```python
import os as _os
_os.environ.setdefault("JAX_PLATFORMS", "cpu")
import jax
import jax.numpy as jnp

def _softmax(x, axis=-1):
    return jax.nn.softmax(x, axis=axis)
def _gelu(x):
    return jax.nn.gelu(x, approximate=True)
def _silu(x):
    return jax.nn.silu(x)
def _sigmoid(x):
    return jax.nn.sigmoid(x)
def _layernorm(x, axis=-1, eps=1e-5):
    m = jnp.mean(x, axis=axis, keepdims=True)
    v = jnp.var(x, axis=axis, keepdims=True)
    return (x - m) / jnp.sqrt(v + eps)
def _scatter_add(tgt, idx, src, axis=0):
    return tgt.at[idx].add(src)
def _segment_sum(src, seg, n):
    return jax.ops.segment_sum(src, seg, n)
class _Rng:
    def __init__(self, key):
        self._k = key
    def _next(self):
        self._k, sub = jax.random.split(self._k)
        return sub
    def normal(self, shape):
        return jax.random.normal(self._next(), shape, dtype=jnp.bfloat16)
    def randint(self, lo, hi, shape):
        return jax.random.randint(self._next(), shape, lo, hi, dtype=jnp.int32)
    def uniform(self, shape, lo=0.0, hi=1.0):
        return jax.random.uniform(self._next(), shape, jnp.bfloat16, lo, hi)
    def permutation(self, n):
        return jax.random.permutation(self._next(), n)


kernel_name = 'concat_heads__compressed_kv_cla__gqa_block_cached__decode'

def setup_inputs():
    _rng = _Rng(jax.random.key(int.from_bytes(__import__("os").urandom(4), "little")))
    _w = (lambda a: (lambda t: t.astype(jnp.bfloat16) if jnp.issubdtype(t.dtype, jnp.floating) else t)(jnp.asarray(a)))
    def _A_setup():
        B, H, Sq, Sk, D, M = 4, 32, 1, 4096, 128, 512
        Dc = 4 * D
        return {
            "x": _w((lambda *s: _rng.normal(s) * 3.2)(B, Sq, M)),
            "c_kv": _w((lambda *s: _rng.normal(s) * 0.05)(B, Sk, Dc)),
            "w_q": _w((lambda *s: _rng.normal(s) * 3.2)(M, H, D) * (M ** -0.5)),
            "w_uk": _w((lambda *s: _rng.normal(s) * 3.2)(Dc, H, D) * (Dc ** -0.5)),
            "w_uv": _w((lambda *s: _rng.normal(s) * 0.05)(Dc, H, D) * (Dc ** -0.5)),
            "w_o": _w((lambda *s: _rng.normal(s) * 0.05)(H, D, M) * ((H * D) ** -0.5)),
        }
    _A_in = _A_setup()

    def _B_setup():
        B, Sq, D = 4, 1, 512
        Hq, Hkv, Sk, Dh = 32, 8, 4096, 128
        assert Hq % Hkv == 0, (Hq, Hkv)
        return {
            "x": _w((lambda *s: _rng.normal(s) * 0.8)(B, Sq, D)),
            "k_cache": _w((lambda *s: _rng.normal(s) * 0.8)(B, Hkv, Sk, Dh)),
            "v_cache": _w((lambda *s: _rng.normal(s) * 0.05)(B, Hkv, Sk, Dh)),
            "wq": _w((lambda *s: _rng.normal(s) * 0.8)(D, Hq * Dh) * (D ** -0.5)),
            "wo": _w((lambda *s: _rng.normal(s) * 0.05)(Hq * Dh, D) * ((Hq * Dh) ** -0.5)),
        }
    _B_in = _B_setup()

    return {
        "A_x": _A_in["x"],
        "A_c_kv": _A_in["c_kv"],
        "A_w_q": _A_in["w_q"],
        "A_w_uk": _A_in["w_uk"],
        "A_w_uv": _A_in["w_uv"],
        "A_w_o": _A_in["w_o"],
        "B_x": _B_in["x"],
        "B_k_cache": _B_in["k_cache"],
        "B_v_cache": _B_in["v_cache"],
        "B_wq": _B_in["wq"],
        "B_wo": _B_in["wo"],
    }

def reference(A_x, A_c_kv, A_w_q, A_w_uk, A_w_uv, A_w_o, B_x, B_k_cache, B_v_cache, B_wq, B_wo):
    def _A_ref(x, c_kv, w_q, w_uk, w_uv, w_o):
        B, Sq, M = x.shape[0], x.shape[1], x.shape[2]
        Sk = c_kv.shape[1]
        H, D = w_q.shape[1], w_q.shape[2]
        q = jnp.einsum("bqm,mhd->bhqd", x, w_q)
        k = jnp.einsum("bkc,chd->bhkd", c_kv, w_uk)
        v = jnp.einsum("bkc,chd->bhkd", c_kv, w_uv)
        scores = jnp.einsum("bhqd,bhkd->bhqk", q, k) * (D ** -0.5)
        off = Sk - Sq
        qi = jnp.arange(Sq)[:, None]
        kj = jnp.arange(Sk)[None, :]
        cmask = kj <= (qi + off)
        scores = jnp.where(cmask[None, None], scores, -1e9)
        p = _softmax(scores, axis=-1)
        ctx = jnp.einsum("bhqk,bhkd->bhqd", p, v)
        return jnp.einsum("bhqd,hdm->bqm", ctx, w_o)

    def _B_ref(x, k_cache, v_cache, wq, wo):
        B, Sq, D = x.shape
        Hq, Dh = 32, 128
        Hkv = k_cache.shape[1]
        rep = Hq // Hkv
        q = (lambda x, *d: x.transpose(*d))((x @ wq).reshape(B, Sq, Hq, Dh), 0, 2, 1, 3)
        k = jnp.repeat(k_cache, rep, axis=1)
        v = jnp.repeat(v_cache, rep, axis=1)
        scores = jnp.einsum("bhqd,bhkd->bhqk", q, k) * (Dh ** -0.5)
        p = _softmax(scores, axis=-1)
        o = jnp.einsum("bhqk,bhkd->bhqd", p, v)
        return (lambda x, *d: x.transpose(*d))(o, 0, 2, 1, 3).reshape(B, Sq, Hq * Dh) @ wo

    a = _A_ref(A_x, A_c_kv, A_w_q, A_w_uk, A_w_uv, A_w_o)
    b = _B_ref(B_x, B_k_cache, B_v_cache, B_wq, B_wo)
    return jnp.concatenate([a, b], axis=-1)
```

```python
import functools

import jax
import jax.numpy as jnp
from jax import lax
import jax.experimental.pallas as pl
import jax.experimental.pallas.tpu as pltpu

F32 = jnp.float32
BF16 = jnp.bfloat16
NT = (((1,), (1,)), ((), ()))
NN = (((1,), (0,)), ((), ()))

B = 4
H = 32
D = 128
M = 512
DC = 512
S = 4096
HKV = 8
NG = B * HKV
PIECE = 512
RING = 4
LAG = 3
HI, LO = 0, 1
SCALE = float(D) ** -0.5


def _dot(a, b, dims=NN):
    return lax.dot_general(a, b, dims, preferred_element_type=F32)


def _iota(shape, dim):
    return lax.broadcasted_iota(jnp.int32, shape, dim)


def _kernel(xa_hbm, ckv_hbm, wqa_hbm, wuk_hbm, wuv_hbm, woa_hbm,
            xb_hbm, k_hbm, v_hbm, wqb_hbm, wob_hbm,
            o_hbm,
            xa_v, xb_v, o_v,
            wqa_v, wuk_v, wuv_v, wqb_v, woa_v, wob_v,
            k_v, v_v, c_v,
            x2_s, r_s, qabs_s, qb_s, qg_s, og_s,
            m_s, l_s, acc_s, lx_s, la_s,
            sem_k, sem_v, sem_c, sem_w, sem_wob, sem_woa, sem_x):

    def rows(i, n):
        if isinstance(i, int):
            return pl.ds(i * n, n)
        return pl.ds(pl.multiple_of(i * n, n), n)

    def cp_n(src, dst, t, sem, prio):
        pltpu.make_async_copy(src.at[rows(t, 128)], dst.at[rows(t, 128)], sem).start(priority=prio)

    def cp_w(src, dst, t, sem, prio):
        pltpu.make_async_copy(src.at[rows(t, 32)], dst.at[rows(t, 32)], sem).start(priority=prio)

    def cp_wqb(t, prio):
        r, c = rows(t // 4, 16), rows(t % 4, 1024)
        pltpu.make_async_copy(wqb_hbm.at[r, c], wqb_v.at[r, c], sem_w.at[2]).start(priority=prio)

    def wait_all(buf, sem):
        pltpu.make_async_copy(buf, buf, sem).wait()

    def tick_kv(g, j):
        s = g & (RING - 1) if not isinstance(g, int) else g % RING
        cp_n(v_hbm.at[g], v_v.at[s], j, sem_v.at[s], LO)
        cp_n(k_hbm.at[g], k_v.at[s], j, sem_k.at[s], HI)

    def tick_c(g, j):
        s = g & (RING - 1) if not isinstance(g, int) else g % RING
        cp_w(ckv_hbm.at[g], c_v.at[s], j + 8, sem_c.at[s], LO)
        cp_w(ckv_hbm.at[g], c_v.at[s], j, sem_c.at[s], HI)

    def tick_wuv(t):
        cp_n(wuv_hbm, wuv_v, t + 64, sem_w.at[3], LO)
        cp_n(wuv_hbm, wuv_v, t, sem_w.at[3], HI)

    def tick_wo(t):
        cp_w(woa_hbm, woa_v, t, sem_woa.at[t // 8], LO)
        cp_w(wob_hbm, wob_v, t, sem_wob.at[t // 32], HI)

    def loop(lo, hi, fn, unroll=1):
        def body(i, c):
            fn(i)
            return c
        lax.fori_loop(lo, hi, body, 0, unroll=unroll)

    def t0(t):
        cp_n(wuk_hbm, wuk_v, t, sem_w.at[1], LO)
        cp_n(wqa_hbm, wqa_v, t, sem_w.at[0], HI)
    t0(0)
    cxa = pltpu.make_async_copy(xa_hbm, xa_v, sem_x.at[0])
    cxb = pltpu.make_async_copy(xb_hbm, xb_v, sem_x.at[1])
    cxa.start()
    cxb.start()
    loop(1, 128, t0)

    cxa.wait()
    cxb.wait()
    ex = (_iota((128, 256), 1) // 2 == _iota((128, 256), 0)).astype(BF16)
    par8 = (_iota((8, 256), 1) % 2) == (_iota((8, 256), 0) // 4)
    xa = xa_v[...].astype(F32)
    xa8 = jnp.concatenate([xa, xa], axis=0).astype(BF16)
    for n in range(4):
        t = _dot(xa8[:, n * 128:(n + 1) * 128], ex)
        t = jnp.where(par8, t, 0.0)
        x2_s[2 * n] = t[:, :128]
        x2_s[2 * n + 1] = t[:, 128:]
    m_s[...] = jnp.full(m_s.shape, -jnp.inf, F32)
    l_s[...] = jnp.zeros(l_s.shape, F32)
    acc_s[...] = jnp.zeros(acc_s.shape, F32)
    qb_s[pl.ds(256, 32), :] = jnp.zeros((32, 128), F32)
    og_s[pl.ds(256, 256), :] = jnp.zeros((256, 128), F32)

    def t1(t):
        cp_wqb(t + 64, LO)
        cp_wqb(t, HI)
    loop(0, 64, t1)

    def tiles(w_v, j):
        w32 = w_v.at[rows(j, 2048)].bitcast(jnp.uint32)
        return [pltpu.bitcast(w32[pl.ds(p, 64, stride=16), :], BF16) for p in range(16)]

    loop(0, 8, lambda j: tick_c(0, j))
    wait_all(wqa_v, sem_w.at[0])

    def qa_job(j, acc):
        for u in range(4):
            tick_kv(0, 4 * j + u)
        return acc + _dot(x2_s[j].astype(BF16), jnp.concatenate(tiles(wqa_v, j), axis=1))
    qa = lax.fori_loop(0, 8, qa_job, jnp.zeros((8, 2048), F32)).astype(BF16)

    loop(0, 8, lambda j: tick_c(1, j))
    wait_all(wuk_v, sem_w.at[1])
    parw = (_iota((128, 128), 1) % 2) == ((_iota((128, 128), 0) // 4) % 2)

    def qabs_job(j):
        for u in range(4):
            tick_kv(1, 4 * j + u)
        tl = tiles(wuk_v, j)
        r = jnp.concatenate([_dot(qa[:, p * 128:(p + 1) * 128], tl[p], NT) for p in range(16)], axis=0)
        r_s[j] = jnp.where(parw, r, 0.0).astype(BF16)
    loop(0, 8, qabs_job)

    cmp = (_iota((256, 128), 0) // 2 == _iota((256, 128), 1)).astype(BF16)
    perm = ((_iota((128, 128), 0) % 32) * 4 + _iota((128, 128), 0) // 32
            == _iota((128, 128), 1)).astype(BF16)
    for n in range(4):
        t = _dot(jnp.concatenate([r_s[2 * n], r_s[2 * n + 1]], axis=1), cmp).astype(BF16)
        qabs_s[:, n * 128:(n + 1) * 128] = _dot(perm, t).astype(BF16)

    loop(0, 8, lambda j: tick_c(2, j))
    wait_all(wqb_v, sem_w.at[2])
    xb = xb_v[...].astype(F32)
    xb8 = jnp.concatenate([xb, xb], axis=0).astype(BF16)

    def qb_job(p):
        tick_kv(2, 2 * p)
        tick_kv(2, 2 * p + 1)
        q = _dot(xb8, wqb_v[:, rows(p, 256)])
        qb_s[rows(2 * p, 8), :] = q[:, :128]
        qb_s[rows(2 * p + 1, 8), :] = q[:, 128:]
    loop(0, 16, qb_job)
    for g in range(NG):
        b, hk = g // HKV, g % HKV
        qg_s[g] = qb_s[pl.ds(hk * 32 + b, 8, stride=8), :]

    def main(i, tick1, tick2):
        s = i & (RING - 1)
        wait_all(k_v.at[s], sem_k.at[s])
        q = qg_s[i].astype(BF16)
        sc = []
        for j in range(8):
            tick1(2 * j)
            tick1(2 * j + 1)
            sc.append(_dot(q, k_v[s, pl.ds(j * 512, 512), :], NT))
        sc = jnp.concatenate(sc, axis=1)
        mx = jnp.max(sc, axis=-1, keepdims=True)
        p = jnp.exp((sc - mx) * SCALE)
        l = jnp.sum(p, axis=-1, keepdims=True)
        p = p.astype(BF16)

        wait_all(c_v.at[s], sem_c.at[s])
        b = i // 8
        qa = qabs_s[rows(b, 32), :]
        sa = []
        for j in range(4):
            tick2(j)
            sa.append(_dot(qa, c_v[s, pl.ds(j * 128, 128), :], NT))
        sa = jnp.concatenate(sa, axis=1)
        m_old = m_s[b]
        m_new = jnp.maximum(m_old, jnp.max(sa, axis=-1, keepdims=True))
        alpha = jnp.exp((m_old - m_new) * SCALE)
        pa = jnp.exp((sa - m_new) * SCALE)
        l_s[b] = alpha * l_s[b] + jnp.sum(pa, axis=-1, keepdims=True)
        m_s[b] = m_new
        pa = pa.astype(BF16)

        wait_all(v_v.at[s], sem_v.at[s])
        o = jnp.zeros((8, 128), F32)
        for j in range(8):
            tick1(16 + 2 * j)
            tick1(16 + 2 * j + 1)
            o = o + _dot(p[:, j * 512:(j + 1) * 512], v_v[s, pl.ds(j * 512, 512), :])
        og_s[rows(i, 8), :] = o / l

        acc = acc_s[b] * alpha
        for j in range(4):
            tick2(4 + j)
            acc = acc + _dot(pa[:, j * 128:(j + 1) * 128], c_v[s, pl.ds(j * 128, 128), :])
        acc_s[b] = acc

    loop(0, NG - LAG, lambda i: main(i, lambda j: tick_kv(i + LAG, j), lambda j: tick_c(i + LAG, j)))
    loop(NG - LAG, NG - 1, lambda i: main(i, lambda j: tick_wuv((i - (NG - LAG)) * 32 + j),
                                          lambda j: tick_wo((i - (NG - LAG)) * 8 + j)))
    main(NG - 1, lambda j: tick_wo(16 + j), lambda j: tick_wo(48 + j))

    ob = jnp.concatenate(
        [og_s[pl.ds((h // 4) * 8 + h % 4, 8, stride=64), :] for h in range(H)], axis=1).astype(BF16)

    permt = ((_iota((128, 128), 1) % 32) * 4 + _iota((128, 128), 1) // 32
             == _iota((128, 128), 0)).astype(BF16)
    par128 = (_iota((128, 256), 1) % 2) == ((_iota((128, 256), 0) // 4) % 2)
    cc = jnp.concatenate([acc_s[b] / l_s[b] for b in range(B)], axis=0).astype(BF16)
    for n in range(4):
        t = _dot(permt, cc[:, n * 128:(n + 1) * 128]).astype(BF16)
        t = jnp.where(par128, _dot(t, ex), 0.0)
        lx_s[2 * n] = t[:, :128]
        lx_s[2 * n + 1] = t[:, 128:]

    loop(56, 80, tick_wo)
    wait_all(wob_v.at[pl.ds(0, 1024)], sem_wob.at[0])
    outb = _dot(ob[:, 0:1024], wob_v[pl.ds(0, 1024), :])
    wait_all(wuv_v, sem_w.at[3])
    top = _iota((8, 128), 0) < 4

    def ctx_job(j, acc):
        for u in range(6):
            tick_wo(80 + 6 * j + u)
        tl = tiles(wuv_v, j)
        return acc + jnp.concatenate(
            [_dot(lx_s[j, pl.ds(p * 8, 8), :].astype(BF16), tl[p]) for p in range(16)], axis=0)
    ctx = lax.fori_loop(0, 8, ctx_job, jnp.zeros((128, 128), F32))
    for p in range(16):
        c = ctx[p * 8:(p + 1) * 8]
        la_s[p] = jnp.concatenate([jnp.where(top, c, 0.0), jnp.where(top, 0.0, c)], axis=1)

    for u in range(1, 4):
        wait_all(wob_v.at[pl.ds(u * 1024, 1024)], sem_wob.at[u])
        outb = outb + _dot(ob[:, u * 1024:(u + 1) * 1024], wob_v[pl.ds(u * 1024, 1024), :])
    o_v[:, M:] = outb[0:4].astype(BF16)

    def woa_job(p, acc):
        blk = woa_v.at[rows(p, 256)]
        wait_all(blk, sem_woa.at[p])
        return acc + _dot(la_s[p].astype(BF16), blk[...])
    outa = lax.fori_loop(0, 16, woa_job, jnp.zeros((8, M), F32))
    o_v[:, :M] = (outa[0:4] + outa[4:8]).astype(BF16)
    co = pltpu.make_async_copy(o_v, o_hbm, sem_x.at[0])
    co.start()
    co.wait()


@jax.jit
def pallas_concat_heads__compressed_kv_cla__gqa_block_cached__decode_kernel(A_x, A_c_kv, A_w_q, A_w_uk, A_w_uv, A_w_o, B_x, B_k_cache, B_v_cache, B_wq, B_wo):
    args = (
        A_x.reshape(B, M),
        A_c_kv.reshape(NG, PIECE, DC),
        A_w_q.reshape(M * H, D),
        A_w_uk.reshape(DC * H, D),
        A_w_uv.reshape(DC * H, D),
        A_w_o.reshape(H * D, M),
        B_x.reshape(B, M),
        B_k_cache.reshape(NG, S, D),
        B_v_cache.reshape(NG, S, D),
        B_wq,
        B_wo,
    )
    V = pltpu.VMEM
    scratch = [
        V((B, M), BF16), V((B, M), BF16), V((B, 2 * M), BF16),
        V((M * H, D), BF16), V((DC * H, D), BF16), V((DC * H, D), BF16),
        V((M, H * D), BF16), V((H * D, M), BF16), V((H * D, M), BF16),
        V((RING, S, D), BF16), V((RING, S, D), BF16), V((RING, PIECE, DC), BF16),
        V((8, 8, 128), F32),
        V((8, 128, 128), BF16),
        V((128, DC), BF16),
        V((256 + 32, D), F32),
        V((NG, 8, D), F32),
        V((512, D), F32),
        V((B, H, 1), F32), V((B, H, 1), F32), V((B, H, DC), F32),
        V((8, 128, 128), F32),
        V((16, 8, 256), F32),
        pltpu.SemaphoreType.DMA((RING,)), pltpu.SemaphoreType.DMA((RING,)),
        pltpu.SemaphoreType.DMA((RING,)), pltpu.SemaphoreType.DMA((4,)),
        pltpu.SemaphoreType.DMA((4,)), pltpu.SemaphoreType.DMA((16,)),
        pltpu.SemaphoreType.DMA((2,)),
    ]
    out = pl.pallas_call(
        _kernel,
        in_specs=[pl.BlockSpec(memory_space=pl.ANY)] * 11,
        out_specs=pl.BlockSpec(memory_space=pl.ANY),
        out_shape=jax.ShapeDtypeStruct((B, 2 * M), BF16),
        scratch_shapes=scratch,
        compiler_params=pltpu.CompilerParams(
            vmem_limit_bytes=64 * 1024 * 1024,
            disable_bounds_checks=True,
            disable_semaphore_checks=True,
        ),
    )(*args)
    return out.reshape(B, 1, 2 * M)
```

```python
import jax
import jax.numpy as jnp
from jax import lax
import jax.experimental.pallas as pl
import jax.experimental.pallas.tpu as pltpu

F32 = jnp.float32
BF16 = jnp.bfloat16
NT = (((1,), (1,)), ((), ()))
NN = (((1,), (0,)), ((), ()))

NOMAIN = False
NOTAIL = False
B = 4
H = 32
D = 128
M = 512
DC = 512
S = 4096
HKV = 8
NIT = 32
RING = 4
LAG = 2
OFF = 2
LASTMODE = 'a'
HI, LO = 0, 1
SCALE = float(D) ** -0.5

S_U, S_WQA, S_WUK, S_WQB, S_WUV, S_X, S_WOB, S_WOA, S_N = 0, 4, 5, 6, 7, 8, 10, 18, 29


def _dot(a, b, dims=NN):
    return lax.dot_general(a, b, dims, preferred_element_type=F32)


def _iota(shape, dim):
    return lax.broadcasted_iota(jnp.int32, shape, dim)


def _kernel(xa_hbm, ckv_hbm, wqa_hbm, wuk_hbm, wuv_hbm, woa_hbm,
            xb_hbm, k_hbm, v_hbm, wqb_hbm, wob_hbm,
            o_hbm,
            xa_v, xb_v, o_v, k_v, v_v, c_v, wqa_v, wuk_v, wuv_v, wqb_v, woa_v, wob_v,
            x2_s, r_s, qabs_s, qb_s, qg_s, og_s, ob_s,
            ma_s, la_s, acca_s, mb_s, lb_s, accb_s, lx_s, lo_s, sem):

    def ds(start, n):
        if isinstance(start, int):
            return pl.ds(start, n)
        return pl.ds(pl.multiple_of(start, n), n)

    def rows(i, n):
        return ds(i * n, n)

    def go(src, dst, s, prio):
        pltpu.make_async_copy(src, dst, sem.at[s]).start(priority=prio)

    def wait_all(buf, s):
        pltpu.make_async_copy(buf, buf, sem.at[s]).wait()

    def loop(lo, hi, fn):
        def body(i, c):
            fn(i)
            return c
        lax.fori_loop(lo, hi, body, 0)

    def cp_n(src, dst, t, s, prio):
        go(src.at[:, rows(t, 32)], dst.at[:, rows(t, 32)], s, prio)

    def tick_p1(t):
        cp_n(wuk_hbm, wuk_v, t, S_WUK, LO)
        cp_n(wqa_hbm, wqa_v, t, S_WQA, HI)

    def tick_p2(t):
        c = rows(t & 7, 512)
        for off, prio in ((8, LO), (0, HI)):
            r = rows((t >> 3) + off, 8)
            go(wqb_hbm.at[:, r, c], wqb_v.at[:, r, c], S_WQB, prio)

    def tick_main(i, j, wrap=False):
        s, w, p = i & (RING - 1), i >> 3, i & 7

        def kv(g0, n, d0, r0, nr):
            rs = pl.ds(pl.multiple_of(p * 512 + j * 64 + r0, 8), nr)
            rd = pl.ds(pl.multiple_of(j * 64 + r0, 8), nr)
            return [(lambda: go(v_hbm.at[pl.ds(g0, n), rs], v_v.at[s, pl.ds(d0, n), rd], S_U + s, LO)),
                    (lambda: go(k_hbm.at[pl.ds(g0, n), rs], k_v.at[s, pl.ds(d0, n), rd], S_U + s, HI))]
        if not wrap or OFF == 0:
            for u in range(4):
                for f in kv(w * 8 + OFF, 8, 0, u * 16, 16):
                    f()
        elif LASTMODE == 'a':
            for r0, nr in ((0, 24), (24, 24), (48, 16)):
                for f in kv(24 + OFF, 8 - OFF, 0, r0, nr):
                    f()
            for f in kv(0, OFF, 8 - OFF, 0, 64):
                f()
        else:
            for u in range(4):
                a, b2 = kv(24 + OFF, 8 - OFF, 0, u * 16, 16), kv(0, OFF, 8 - OFF, u * 16, 16)
                a[0](); b2[0](); a[1](); b2[1]()
        go(ckv_hbm.at[w, rows(64 + p * 8 + j, 32)], c_v.at[s, rows(8 + j, 32)], S_U + s, LO)
        go(ckv_hbm.at[w, rows(p * 8 + j, 32)], c_v.at[s, rows(j, 32)], S_U + s, HI)

    def tick_e1(t):
        cp_n(wuv_hbm, wuv_v, t + 64, S_WUV, LO)
        cp_n(wuv_hbm, wuv_v, t, S_WUV, HI)

    def tick_e2(t):
        fin = t >= 112
        q = jnp.where(fin, (t >> 2) & 3, t & 3)
        r = rows(jnp.where(fin, 28 + (t & 3), t >> 2), 32)
        go(woa_hbm.at[q, r], woa_v.at[q, r], S_WOA + jnp.where(fin, 7 + q, t >> 4), LO)
        go(wob_hbm.at[:, rows(t, 8)], wob_v.at[:, rows(t, 8)], S_WOB + (t >> 4), HI)

    tick_p1(0)
    cxa = pltpu.make_async_copy(xa_hbm, xa_v, sem.at[S_X])
    cxb = pltpu.make_async_copy(xb_hbm, xb_v, sem.at[S_X + 1])
    cxa.start()
    cxb.start()
    loop(1, 64, tick_p1)

    cxa.wait()
    cxb.wait()
    ex = (_iota((128, 256), 1) // 2 == _iota((128, 256), 0)).astype(BF16)
    par8 = (_iota((8, 256), 1) % 2) == (_iota((8, 256), 0) // 4)
    xa = xa_v[...].astype(F32)
    xa8 = jnp.concatenate([xa, xa], axis=0).astype(BF16)
    for n in range(4):
        t = _dot(xa8[:, n * 128:(n + 1) * 128], ex)
        t = jnp.where(par8, t, 0.0)
        x2_s[2 * n] = t[:, :128]
        x2_s[2 * n + 1] = t[:, 128:]

    def init(b):
        ma_s[b] = jnp.full(ma_s.shape[1:], -jnp.inf, F32)
        la_s[b] = jnp.zeros(la_s.shape[1:], F32)
        acca_s[b] = jnp.zeros(acca_s.shape[1:], F32)
        mb_s[b] = jnp.full(mb_s.shape[1:], -jnp.inf, F32)
        lb_s[b] = jnp.zeros(lb_s.shape[1:], F32)
        accb_s[b] = jnp.zeros(accb_s.shape[1:], F32)
        qb_s[rows(32 + b, 8), :] = jnp.zeros((8, 128), F32)
        og_s[rows(4 + b, 64), :] = jnp.zeros((64, 128), F32)
    loop(0, B, init)

    loop(64, 128, tick_p1)
    loop(0, 32, tick_p2)

    def tile(w_v, j, p):
        w32 = w_v.at[j >> 1, rows(j & 1, 2048)].bitcast(jnp.uint32)
        return pltpu.bitcast(w32[pl.ds(p, 64, stride=16), :], BF16)

    wait_all(wqa_v, S_WQA)

    def qa_job(j, acc):
        loop(32 + 4 * j, 36 + 4 * j, tick_p2)
        return acc + _dot(x2_s[j].astype(BF16), jnp.concatenate([tile(wqa_v, j, p) for p in range(16)], axis=1))
    qa = lax.fori_loop(0, 8, qa_job, jnp.zeros((8, 2048), F32)).astype(BF16)

    wait_all(wuk_v, S_WUK)
    parw = (_iota((128, 128), 1) % 2) == ((_iota((128, 128), 0) // 4) % 2)

    def qabs_job(j):
        tick_main(0, j)
        r = [_dot(qa[:, p * 128:(p + 1) * 128], tile(wuk_v, j, p), NT) for p in range(16)]
        r_s[j] = jnp.where(parw, jnp.concatenate(r, axis=0), 0.0).astype(BF16)
    loop(0, 8, qabs_job)

    cmp = (_iota((256, 128), 0) // 2 == _iota((256, 128), 1)).astype(BF16)
    perm = ((_iota((128, 128), 0) % 32) * 4 + _iota((128, 128), 0) // 32
            == _iota((128, 128), 1)).astype(BF16)

    def pack_job(n):
        t = _dot(jnp.concatenate([r_s[2 * n], r_s[2 * n + 1]], axis=1), cmp).astype(BF16)
        qabs_s[n] = _dot(perm, t).astype(BF16)
    loop(0, 4, pack_job)

    wait_all(wqb_v, S_WQB)
    xb = xb_v[...].astype(F32)
    xb8 = jnp.concatenate([xb, xb], axis=0).astype(BF16)

    def qb_job(j):
        tick_main(1, j)
        q = _dot(xb8, wqb_v[:, :, rows(j, 512)].reshape(M, 512))
        for u in range(4):
            qb_s[rows(4 * j + u, 8), :] = q[:, u * 128:(u + 1) * 128]
    loop(0, 8, qb_job)
    for w in range(4):
        for r in range(8):
            g = (8 * w + OFF + r) % 32
            qg_s[w, pl.ds(r * 8, 8), :] = qb_s[pl.ds((g % 8) * 32 + g // 8, 8, stride=8), :]

    def online(sc, m_s, l_s, b):
        m_old = m_s[b]
        m_new = jnp.maximum(m_old, jnp.max(sc, axis=-1, keepdims=True))
        alpha = jnp.exp((m_old - m_new) * SCALE)
        p = jnp.exp((sc - jnp.tile(m_new, (1, 4))) * SCALE)
        l_s[b] = alpha * l_s[b] + ((p[:, 0:128] + p[:, 128:256]) + (p[:, 256:384] + p[:, 384:512]))
        m_s[b] = m_new
        return p, alpha

    def main(i):
        @pl.when(i < 24 - LAG)
        def _():
            loop(0, 8, lambda j: tick_main(i + LAG, j))

        @pl.when(jnp.logical_and(i >= 24 - LAG, i < NIT - LAG))
        def _():
            loop(0, 8, lambda j: tick_main(i + LAG, j, True))

        @pl.when(i >= NIT - LAG)
        def _():
            e = i - (NIT - LAG)
            loop(e * 24, 24 + e * 28, tick_e1)

        s, b = i & (RING - 1), i >> 3
        wait_all(k_v.at[s], S_U + s)
        wait_all(v_v.at[s], S_U + s)
        wait_all(c_v.at[s], S_U + s)
        if NOMAIN:
            return
        sc = [_dot(qg_s[b, pl.ds(g * 8, 8), :].astype(BF16), k_v[s, g], NT) for g in range(HKV)]
        p, alpha = online(jnp.concatenate(sc, axis=0), mb_s, lb_s, b)

        qa = jnp.concatenate([qabs_s[n, rows(b, 32), :] for n in range(4)], axis=1)
        pa, alpha_a = online(_dot(qa, c_v[s], NT), ma_s, la_s, b)

        o = [_dot(p[g * 8:(g + 1) * 8].astype(BF16), v_v[s, g]) for g in range(HKV)]
        accb_s[b] = accb_s[b] * alpha + jnp.concatenate(o, axis=0)
        acca_s[b] = acca_s[b] * jnp.tile(alpha_a, (1, 4)) + _dot(pa.astype(BF16), c_v[s])

    loop(0, NIT, main)

    loop(52, 64, tick_e1)
    for b in range(B):
        o = accb_s[b] / jnp.sum(lb_s[b], axis=-1, keepdims=True)
        if b < 3 or OFF == 0:
            og_s[pl.ds(b * 64 + OFF * 8, 64), :] = o
        else:
            og_s[pl.ds(192 + OFF * 8, 64 - OFF * 8), :] = o[:64 - OFF * 8]
            og_s[pl.ds(0, OFF * 8), :] = o[64 - OFF * 8:]
        acca_s[b] = acca_s[b] / jnp.sum(la_s[b], axis=-1, keepdims=True)
    for h in range(H):
        ob_s[h % 8, :, pl.ds((h // 8) * 128, 128)] = og_s[pl.ds((h // 4) * 8 + h % 4, 8, stride=64), :]

    permt = ((_iota((128, 128), 1) % 32) * 4 + _iota((128, 128), 1) // 32
             == _iota((128, 128), 0)).astype(BF16)
    par128 = (_iota((128, 256), 1) % 2) == ((_iota((128, 256), 0) // 4) % 2)

    def expand_job(n):
        loop(n * 12, n * 12 + 12, tick_e2)
        cc = acca_s[:, :, rows(n, 128)].reshape(128, 128).astype(BF16)
        t = _dot(permt, cc).astype(BF16)
        t = jnp.where(par128, _dot(t, ex), 0.0)
        lx_s[2 * n] = t[:, :128]
        lx_s[2 * n + 1] = t[:, 128:]
    loop(0, 4, expand_job)

    wait_all(wuv_v, S_WUV)
    top = _iota((8, 128), 0) < 4

    def ctx_job(j, acc):
        loop(48 + 4 * j, 52 + 4 * j, tick_e2)
        return acc + jnp.concatenate(
            [_dot(lx_s[j, pl.ds(p * 8, 8), :].astype(BF16), tile(wuv_v, j, p)) for p in range(16)], axis=0)
    ctx = lax.fori_loop(0, 8, ctx_job, jnp.zeros((128, 128), F32))
    for h in range(H):
        c = ctx[(h // 2) * 8:(h // 2) * 8 + 8]
        if h % 8 == 7:
            c = pltpu.roll(c, 4, 0)
        else:
            c = jnp.where(top, c, 0.0) if h % 2 == 0 else jnp.where(top, 0.0, c)
        lo_s[h % 8, :, pl.ds((h // 8) * 128, 128)] = c

    def proj(lhs_s, w_v, a, s):
        blk = w_v.at[:, rows(a, 128)]
        lhs = lhs_s[a].astype(BF16)
        wait_all(blk, s)
        return _dot(lhs, blk[...].reshape(512, M))

    def wo_job(a, carry):
        outa, outb = carry
        loop(jnp.clip(64 + 16 * a, 80, 128), jnp.clip(80 + 16 * a, 80, 128), tick_e2)
        outb = outb + proj(ob_s, wob_v, a + 1, S_WOB + a + 1)
        outa = outa + proj(lo_s, woa_v, a, S_WOA + a)
        return outa, outb
    outa, outb = lax.fori_loop(0, 7, wo_job, (jnp.zeros((8, M), F32), proj(ob_s, wob_v, 0, S_WOB)))
    o_v[:, M:] = outb[0:4].astype(BF16)
    outa = outa + pltpu.roll(outa, 4, 0)

    def fin_job(q, acc):
        blk = woa_v.at[q, pl.ds(896, 128)]
        lhs = lo_s[7, :, rows(q, 128)].astype(BF16)
        wait_all(blk, S_WOA + 7 + q)
        if NOTAIL:
            return acc
        return acc + _dot(lhs, blk[...])
    outa = lax.fori_loop(0, 4, fin_job, outa)
    o_v[:, :M] = outa[0:4].astype(BF16)
    co = pltpu.make_async_copy(o_v, o_hbm, sem.at[S_X])
    co.start()
    co.wait()


@jax.jit
def pallas_concat_heads__compressed_kv_cla__gqa_block_cached__decode_kernel(A_x, A_c_kv, A_w_q, A_w_uk, A_w_uv, A_w_o, B_x, B_k_cache, B_v_cache, B_wq, B_wo):
    args = (
        A_x.reshape(B, M),
        A_c_kv,
        A_w_q.reshape(4, 4096, D),
        A_w_uk.reshape(4, 4096, D),
        A_w_uv.reshape(4, 4096, D),
        A_w_o.reshape(4, 1024, M),
        B_x.reshape(B, M),
        B_k_cache.reshape(B * HKV, S, D),
        B_v_cache.reshape(B * HKV, S, D),
        B_wq.reshape(4, 128, H * D),
        B_wo.reshape(4, 1024, M),
    )
    V = pltpu.VMEM
    scratch = [
        V((B, M), BF16), V((B, M), BF16), V((B, 2 * M), BF16),
        V((RING, HKV, 512, D), BF16), V((RING, HKV, 512, D), BF16), V((RING, 512, DC), BF16),
        V((4, 4096, D), BF16), V((4, 4096, D), BF16), V((4, 4096, D), BF16),
        V((4, 128, H * D), BF16), V((4, 1024, M), BF16), V((4, 1024, M), BF16),
        V((8, 8, 128), F32),
        V((8, 128, 128), BF16),
        V((4, 128, 128), BF16),
        V((256 + 32, D), F32),
        V((B, 64, D), F32),
        V((512, D), F32),
        V((8, 8, 512), F32),
        V((B, H, 128), F32), V((B, H, 128), F32), V((B, H, DC), F32),
        V((B, 64, 128), F32), V((B, 64, 128), F32), V((B, 64, D), F32),
        V((8, 128, 128), F32),
        V((8, 8, 512), F32),
        pltpu.SemaphoreType.DMA((S_N,)),
    ]
    out = pl.pallas_call(
        _kernel,
        in_specs=[pl.BlockSpec(memory_space=pl.ANY)] * 11,
        out_specs=pl.BlockSpec(memory_space=pl.ANY),
        out_shape=jax.ShapeDtypeStruct((B, 2 * M), BF16),
        scratch_shapes=scratch,
        compiler_params=pltpu.CompilerParams(
            vmem_limit_bytes=64 * 1024 * 1024,
            disable_bounds_checks=True,
            disable_semaphore_checks=True,
        ),
    )(*args)
    return out.reshape(B, 1, 2 * M)
```

```python
import jax
import jax.numpy as jnp
from jax import lax
import jax.experimental.pallas as pl
import jax.experimental.pallas.tpu as pltpu

F32 = jnp.float32
BF16 = jnp.bfloat16
NT = (((1,), (1,)), ((), ()))
NN = (((1,), (0,)), ((), ()))

B = 4
H = 32
D = 128
M = 512
DC = 512
S = 4096
HKV = 8
NIT = 32
RING = 4
LAG = 3
OFF = 2
SH = 8
HI, LO = 0, 1
SCALE = float(D) ** -0.5

S_K, S_V, S_C, S_WQA, S_WUK, S_WQB, S_WUV, S_X, S_WOB, S_WOA, S_N = (
    0, 4, 8, 12, 13, 14, 15, 16, 18, 26, 37)


def _dot(a, b, dims=NN):
    return lax.dot_general(a, b, dims, preferred_element_type=F32)


def _iota(shape, dim):
    return lax.broadcasted_iota(jnp.int32, shape, dim)


def _kernel(xa_hbm, ckv_hbm, wqa_hbm, wuk_hbm, wuv_hbm, woa_hbm,
            xb_hbm, k_hbm, v_hbm, wqb_hbm, wob_hbm,
            o_hbm,
            xa_v, xb_v, o_v, k_v, v_v, c_v, wqa_v, wuk_v, wuv_v, wqb_v, woa_v, wob_v,
            x2_s, r_s, qabs_s, qb_s, qg_s, og_s, ob_s,
            ma_s, la_s, acca_s, mb_s, lb_s, accb_s, lx_s, lo_s, w32_s, sem):

    def ds(start, n, align):
        if isinstance(start, int):
            return pl.ds(start, n)
        return pl.ds(pl.multiple_of(start, align), n)

    def rows(i, n):
        return ds(i * n, n, n)

    def go(src, dst, s, prio):
        pltpu.make_async_copy(src, dst, sem.at[s]).start(priority=prio)

    def wait_all(buf, s):
        pltpu.make_async_copy(buf, buf, sem.at[s]).wait()

    def loop(lo, hi, fn):
        def body(i, c):
            fn(i)
            return c
        lax.fori_loop(lo, hi, body, 0)

    def cp_n(src, dst, half, t, s, prio):
        g = pl.ds(half * 4, 4)
        go(src.at[g, rows(t, 16)], dst.at[g, rows(t, 16)], s, prio)

    def cp_q(half, t, prio):
        g, r, c = pl.ds(half * 4, 4), rows(t >> 4, 8), rows(t & 15, 256)
        go(wqb_hbm.at[g, r, c], wqb_v.at[g, r, c], S_WQB, prio)

    def tick_pa(t):
        cp_n(wqa_hbm, wqa_v, 1, t, S_WQA, LO)
        cp_q(0, t, LO)
        cp_n(wuv_hbm, wuv_v, 0, t, S_WUV, HI)
        cp_q(1, t, HI)

    def tick_pb(t):
        cp_n(wuk_hbm, wuk_v, 0, t, S_WUK, LO)
        cp_n(wuv_hbm, wuv_v, 1, t, S_WUV, LO)
        cp_n(wqa_hbm, wqa_v, 0, t, S_WQA, HI)
        cp_n(wuk_hbm, wuk_v, 1, t, S_WUK, HI)

    def tick_main(i, j, wrap=False):
        s, w, p = i & (RING - 1), i >> 3, i & 7

        def cp(is_k, g0, n, d0, u, prio):
            src, dst, sm = (k_hbm, k_v, S_K) if is_k else (v_hbm, v_v, S_V)
            a = j * 64 + u * 16
            segs = [(p * 512 + a + SH, a, 16)]
            if isinstance(j, int) and a == 496:
                segs = [(p * 512 + a + SH, a, 16 - SH), ((p * 512 + 512) & (S - 1), 512 - SH, SH)]
            for rs, rd, nr in segs:
                go(src.at[pl.ds(g0, n), ds(rs, nr, 8)], dst.at[s, pl.ds(d0, n), ds(rd, nr, 8)],
                   sm + s, prio)

        for u in range(4):
            if not wrap:
                cp(False, w * 8 + OFF, 8, 0, u, LO)
                cp(True, w * 8 + OFF, 8, 0, u, HI)
            else:
                cp(False, 24 + OFF, 8 - OFF, 0, u, LO)
                cp(True, 0, OFF, 8 - OFF, u, LO)
                cp(True, 24 + OFF, 8 - OFF, 0, u, HI)
                cp(False, 0, OFF, 8 - OFF, u, HI)
        go(ckv_hbm.at[w, rows(64 + p * 8 + j, 32)], c_v.at[s, rows(8 + j, 32)], S_C + s, LO)
        go(ckv_hbm.at[w, rows(p * 8 + j, 32)], c_v.at[s, rows(j, 32)], S_C + s, HI)

    def issue_unit(i, wrap):
        loop(0, 7, lambda j: tick_main(i, j, wrap))
        tick_main(i, 7, wrap)

    def tick_e(t):
        fin = t >= 112
        q = jnp.where(fin, (t >> 2) & 3, t & 3)
        r = rows(jnp.where(fin, 28 + (t & 3), t >> 2), 32)
        go(woa_hbm.at[q, r], woa_v.at[q, r], S_WOA + jnp.where(fin, 7 + q, t >> 4), LO)
        go(wob_hbm.at[:, rows(t, 8)], wob_v.at[:, rows(t, 8)], S_WOB + (t >> 4), HI)

    tick_pa(0)
    cxa = pltpu.make_async_copy(xa_hbm, xa_v, sem.at[S_X])
    cxb = pltpu.make_async_copy(xb_hbm, xb_v, sem.at[S_X + 1])
    cxa.start()
    cxb.start()
    loop(1, 64, tick_pa)

    cxa.wait()
    cxb.wait()
    ex = (_iota((128, 256), 1) // 2 == _iota((128, 256), 0)).astype(BF16)
    par8 = (_iota((8, 256), 1) % 2) == (_iota((8, 256), 0) // 4)
    xa = xa_v[...].astype(F32)
    xa8 = jnp.concatenate([xa, xa], axis=0).astype(BF16)
    for n in range(4):
        t = jnp.where(par8, _dot(xa8[:, n * 128:(n + 1) * 128], ex), 0.0)
        x2_s[2 * n] = t[:, :128]
        x2_s[2 * n + 1] = t[:, 128:]

    def init(b):
        ma_s[b] = jnp.full(ma_s.shape[1:], -jnp.inf, F32)
        la_s[b] = jnp.zeros(la_s.shape[1:], F32)
        acca_s[b] = jnp.zeros(acca_s.shape[1:], F32)
        mb_s[b] = jnp.full(mb_s.shape[1:], -jnp.inf, F32)
        lb_s[b] = jnp.zeros(lb_s.shape[1:], F32)
        accb_s[b] = jnp.zeros(accb_s.shape[1:], F32)
        qb_s[rows(32 + b, 8), :] = jnp.zeros((8, 128), F32)
        og_s[rows(4 + b, 64), :] = jnp.zeros((64, 128), F32)
    loop(0, B, init)

    loop(64, 128, tick_pa)
    loop(0, 40, tick_pb)

    wait_all(wqb_v, S_WQB)
    xb = xb_v[...].astype(F32)
    xb8 = jnp.concatenate([xb, xb], axis=0).astype(BF16)

    def qb_job(j):
        loop(40 + 4 * j, 44 + 4 * j, tick_pb)
        q = _dot(xb8, wqb_v[:, :, rows(j, 512)].reshape(M, 512))
        for u in range(4):
            qb_s[rows(4 * j + u, 8), :] = q[:, u * 128:(u + 1) * 128]
    loop(0, 8, qb_job)
    for w in range(4):
        for r in range(8):
            g = (8 * w + OFF + r) % 32
            qg_s[w, pl.ds(r * 8, 8), :] = qb_s[pl.ds((g % 8) * 32 + g // 8, 8, stride=8), :]
    loop(72, 128, tick_pb)
    loop(0, 8, lambda j: tick_main(0, j))

    def stage(w_v, j):
        w32_s[...] = pltpu.bitcast(w_v[j], jnp.uint32)

    def tile(p):
        return pltpu.bitcast(w32_s[pl.ds(p, 64, stride=16), :], BF16)

    wait_all(wqa_v, S_WQA)

    def qa_job(j, acc):
        tick_main(1, j)
        stage(wqa_v, j)
        w = jnp.concatenate([tile(p) for p in range(16)], axis=1)
        return acc + _dot(x2_s[j].astype(BF16), w)
    qa = lax.fori_loop(0, 8, qa_job, jnp.zeros((8, 2048), F32)).astype(BF16)

    wait_all(wuk_v, S_WUK)
    parw = (_iota((128, 128), 1) % 2) == ((_iota((128, 128), 0) // 4) % 2)

    def qabs_job(j):
        tick_main(2, j)
        stage(wuk_v, j)
        r = [_dot(qa[:, p * 128:(p + 1) * 128], tile(p), NT) for p in range(16)]
        r_s[j] = jnp.where(parw, jnp.concatenate(r, axis=0), 0.0).astype(BF16)
    loop(0, 8, qabs_job)

    cmp = (_iota((256, 128), 0) // 2 == _iota((256, 128), 1)).astype(BF16)
    perm = ((_iota((128, 128), 0) % 32) * 4 + _iota((128, 128), 0) // 32
            == _iota((128, 128), 1)).astype(BF16)

    def pack_job(n):
        t = _dot(jnp.concatenate([r_s[2 * n], r_s[2 * n + 1]], axis=1), cmp).astype(BF16)
        qabs_s[n] = _dot(perm, t).astype(BF16)
    loop(0, 4, pack_job)

    def online(sc, m_s, l_s, b):
        m_old = m_s[b]
        m_new = jnp.maximum(m_old, jnp.max(sc, axis=-1, keepdims=True))
        alpha = jnp.exp((m_old - m_new) * SCALE)
        p = jnp.exp((sc - jnp.tile(m_new, (1, 4))) * SCALE)
        l_s[b] = alpha * l_s[b] + ((p[:, 0:128] + p[:, 128:256]) + (p[:, 256:384] + p[:, 384:512]))
        m_s[b] = m_new
        return p, alpha

    def main(i):
        @pl.when(i < 24 - LAG)
        def _():
            issue_unit(i + LAG, False)

        @pl.when(jnp.logical_and(i >= 24 - LAG, i < NIT - LAG))
        def _():
            issue_unit(i + LAG, True)

        @pl.when(i >= NIT - LAG)
        def _():
            e = i - (NIT - LAG)
            loop(e * 18, e * 18 + 18, tick_e)

        @pl.when(i < 8)
        def _():
            stage(wuv_v, i)
            for p in range(16):
                wuv_v[i, pl.ds(p * 128, 128), :] = tile(p)

        s, b = i & (RING - 1), i >> 3
        wait_all(k_v.at[s], S_K + s)
        wait_all(v_v.at[s], S_V + s)
        wait_all(c_v.at[s], S_C + s)
        sc = [_dot(qg_s[b, pl.ds(g * 8, 8), :].astype(BF16), k_v[s, g], NT) for g in range(HKV)]
        p, alpha = online(jnp.concatenate(sc, axis=0), mb_s, lb_s, b)

        q = jnp.concatenate([qabs_s[n, rows(b, 32), :] for n in range(4)], axis=1)
        pa, alpha_a = online(_dot(q, c_v[s], NT), ma_s, la_s, b)

        o = [_dot(p[g * 8:(g + 1) * 8].astype(BF16), v_v[s, g]) for g in range(HKV)]
        accb_s[b] = accb_s[b] * alpha + jnp.concatenate(o, axis=0)
        acca_s[b] = acca_s[b] * jnp.tile(alpha_a, (1, 4)) + _dot(pa.astype(BF16), c_v[s])

    wait_all(wuv_v, S_WUV)
    loop(0, NIT, main)

    for b in range(B):
        o = accb_s[b] / jnp.sum(lb_s[b], axis=-1, keepdims=True)
        if b < 3:
            og_s[pl.ds(b * 64 + OFF * 8, 64), :] = o
        else:
            og_s[pl.ds(192 + OFF * 8, 64 - OFF * 8), :] = o[:64 - OFF * 8]
            og_s[pl.ds(0, OFF * 8), :] = o[64 - OFF * 8:]
        acca_s[b] = acca_s[b] / jnp.sum(la_s[b], axis=-1, keepdims=True)
    for h in range(H):
        ob_s[h % 8, :, pl.ds((h // 8) * 128, 128)] = (
            og_s[pl.ds((h // 4) * 8 + h % 4, 8, stride=64), :])

    permt = ((_iota((128, 128), 1) % 32) * 4 + _iota((128, 128), 1) // 32
             == _iota((128, 128), 0)).astype(BF16)
    par128 = (_iota((128, 256), 1) % 2) == ((_iota((128, 256), 0) // 4) % 2)

    def expand_job(n):
        loop(54 + n * 4, 58 + n * 4, tick_e)
        cc = acca_s[:, :, rows(n, 128)].reshape(128, 128).astype(BF16)
        t = jnp.where(par128, _dot(_dot(permt, cc).astype(BF16), ex), 0.0)
        lx_s[2 * n] = t[:, :128]
        lx_s[2 * n + 1] = t[:, 128:]
    loop(0, 4, expand_job)

    def ctx_job(j, acc):
        loop(70 + 2 * j, 72 + 2 * j, tick_e)
        return acc + jnp.concatenate(
            [_dot(lx_s[j, pl.ds(p * 8, 8), :].astype(BF16), wuv_v[j, pl.ds(p * 128, 128), :])
             for p in range(16)], axis=0)
    ctx = lax.fori_loop(0, 8, ctx_job, jnp.zeros((128, 128), F32))
    top = _iota((8, 128), 0) < 4
    for h in range(H):
        c = ctx[(h // 2) * 8:(h // 2) * 8 + 8]
        if h % 8 == 7:
            c = pltpu.roll(c, 4, 0)
        else:
            c = jnp.where(top, c, 0.0) if h % 2 == 0 else jnp.where(top, 0.0, c)
        lo_s[h % 8, :, pl.ds((h // 8) * 128, 128)] = c

    def proj(lhs_s, w_v, a, s):
        blk = w_v.at[:, rows(a, 128)]
        lhs = lhs_s[a].astype(BF16)
        wait_all(blk, s)
        return _dot(lhs, blk[...].reshape(512, M))

    def wo_job(a, carry):
        outa, outb = carry
        loop(jnp.minimum(86 + 11 * a, 128), jnp.minimum(97 + 11 * a, 128), tick_e)
        outb = outb + proj(ob_s, wob_v, a + 1, S_WOB + a + 1)
        outa = outa + proj(lo_s, woa_v, a, S_WOA + a)
        return outa, outb
    outa, outb = lax.fori_loop(0, 7, wo_job, (jnp.zeros((8, M), F32), proj(ob_s, wob_v, 0, S_WOB)))
    o_v[:, M:] = outb[0:4].astype(BF16)
    outa = outa + pltpu.roll(outa, 4, 0)

    def fin_job(q, acc):
        blk = woa_v.at[q, pl.ds(896, 128)]
        lhs = lo_s[7, :, rows(q, 128)].astype(BF16)
        wait_all(blk, S_WOA + 7 + q)
        return acc + _dot(lhs, blk[...])
    outa = lax.fori_loop(0, 4, fin_job, outa)
    o_v[:, :M] = outa[0:4].astype(BF16)
    co = pltpu.make_async_copy(o_v, o_hbm, sem.at[S_X])
    co.start()
    co.wait()


@jax.jit
def pallas_concat_heads__compressed_kv_cla__gqa_block_cached__decode_kernel(A_x, A_c_kv, A_w_q, A_w_uk, A_w_uv, A_w_o, B_x, B_k_cache, B_v_cache, B_wq, B_wo):
    args = (
        A_x.reshape(B, M),
        A_c_kv,
        A_w_q.reshape(8, 2048, D),
        A_w_uk.reshape(8, 2048, D),
        A_w_uv.reshape(8, 2048, D),
        A_w_o.reshape(4, 1024, M),
        B_x.reshape(B, M),
        B_k_cache.reshape(B * HKV, S, D),
        B_v_cache.reshape(B * HKV, S, D),
        B_wq.reshape(8, 64, H * D),
        B_wo.reshape(4, 1024, M),
    )
    V = pltpu.VMEM
    scratch = [
        V((B, M), BF16), V((B, M), BF16), V((B, 2 * M), BF16),
        V((RING, HKV, 512, D), BF16), V((RING, HKV, 512, D), BF16), V((RING, 512, DC), BF16),
        V((8, 2048, D), BF16), V((8, 2048, D), BF16), V((8, 2048, D), BF16),
        V((8, 64, H * D), BF16), V((4, 1024, M), BF16), V((4, 1024, M), BF16),
        V((8, 8, 128), F32),
        V((8, 128, 128), BF16),
        V((4, 128, 128), BF16),
        V((256 + 32, D), F32),
        V((B, 64, D), F32),
        V((512, D), F32),
        V((8, 8, 512), F32),
        V((B, H, 128), F32), V((B, H, 128), F32), V((B, H, DC), F32),
        V((B, 64, 128), F32), V((B, 64, 128), F32), V((B, 64, D), F32),
        V((8, 128, 128), F32),
        V((8, 8, 512), F32),
        V((1024, 128), jnp.uint32),
        pltpu.SemaphoreType.DMA((S_N,)),
    ]
    out = pl.pallas_call(
        _kernel,
        in_specs=[pl.BlockSpec(memory_space=pl.ANY)] * 11,
        out_specs=pl.BlockSpec(memory_space=pl.ANY),
        out_shape=jax.ShapeDtypeStruct((B, 2 * M), BF16),
        scratch_shapes=scratch,
        compiler_params=pltpu.CompilerParams(
            vmem_limit_bytes=64 * 1024 * 1024,
            disable_bounds_checks=True,
            disable_semaphore_checks=True,
        ),
    )(*args)
    return out.reshape(B, 1, 2 * M)
```

```python
import jax
import jax.numpy as jnp
from jax import lax
import jax.experimental.pallas as pl
import jax.experimental.pallas.tpu as pltpu

F32 = jnp.float32
BF16 = jnp.bfloat16
NT = (((1,), (1,)), ((), ()))
NN = (((1,), (0,)), ((), ()))

B = 4
H = 32
D = 128
M = 512
DC = 512
S = 4096
HKV = 8
NIT = 32
RING = 4
LAG = 3
OFF = 2
SH = 8
HI, LO = 0, 1
PRE = 7
SCALE = 0.08837890625

S_K, S_V, S_C, S_WQA, S_WUK, S_WQB, S_WUV, S_X, S_WOB, S_WOA, S_N = (
    0, 4, 8, 12, 13, 14, 15, 16, 18, 26, 37)


def _dot(a, b, dims=NN):
    return lax.dot_general(a, b, dims, preferred_element_type=F32)


def _iota(shape, dim):
    return lax.broadcasted_iota(jnp.int32, shape, dim)


def _kernel(xa_hbm, ckv_hbm, wqa_hbm, wuk_hbm, wuv_hbm, woa_hbm,
            xb_hbm, k_hbm, v_hbm, wqb_hbm, wob_hbm,
            o_hbm,
            xa_v, xb_v, o_v, k_v, v_v, c_v, wqa_v, wuk_v, wuv_v, wqb_v, woa_v, wob_v,
            x2_s, r_s, qabs_s, qb_s, qg_s, og_s, ob_s,
            ma_s, la_s, acca_s, mb_s, lb_s, accb_s, lx_s, lo_s, w32_s, sem):

    def ds(start, n, align):
        if isinstance(start, int):
            return pl.ds(start, n)
        return pl.ds(pl.multiple_of(start, align), n)

    def rows(i, n):
        return ds(i * n, n, n)

    def go(src, dst, s, prio):
        pltpu.make_async_copy(src, dst, sem.at[s]).start(priority=prio)

    def wait_all(buf, s):
        pltpu.make_async_copy(buf, buf, sem.at[s]).wait()

    def loop(lo, hi, fn):
        def body(i, c):
            fn(i)
            return c
        lax.fori_loop(lo, hi, body, 0)

    def cp_n(src, dst, half, t, s, prio):
        g = pl.ds(half * 4, 4)
        go(src.at[g, rows(t, 16)], dst.at[g, rows(t, 16)], s, prio)

    def cp_q(half, t, prio):
        g, r, c = pl.ds(half * 4, 4), rows(t >> 4, 8), rows(t & 15, 256)
        go(wqb_hbm.at[g, r, c], wqb_v.at[g, r, c], S_WQB, prio)

    def tick_pa(t, hi=HI):
        cp_n(wqa_hbm, wqa_v, 1, t, S_WQA, LO)
        cp_q(0, t, LO)
        cp_n(wuv_hbm, wuv_v, 0, t, S_WUV, hi)
        cp_q(1, t, hi)

    def tick_pb(t):
        cp_n(wuk_hbm, wuk_v, 0, t, S_WUK, LO)
        cp_n(wuv_hbm, wuv_v, 1, t, S_WUV, LO)
        cp_n(wqa_hbm, wqa_v, 0, t, S_WQA, HI)
        cp_n(wuk_hbm, wuk_v, 1, t, S_WUK, HI)

    def tick_main(i, j, wrap=False):
        s, w, p = i & (RING - 1), i >> 3, i & 7

        def cp(is_k, g0, n, d0, u, prio):
            src, dst, sm = (k_hbm, k_v, S_K) if is_k else (v_hbm, v_v, S_V)
            a = j * 64 + u * 16
            segs = [(p * 512 + a + SH, a, 16)]
            if isinstance(j, int) and a == 496:
                segs = [(p * 512 + a + SH, a, 16 - SH), ((p * 512 + 512) & (S - 1), 512 - SH, SH)]
            for rs, rd, nr in segs:
                go(src.at[pl.ds(g0, n), ds(rs, nr, 8)], dst.at[s, pl.ds(d0, n), ds(rd, nr, 8)],
                   sm + s, prio)

        for u in range(4):
            if not wrap:
                cp(False, w * 8 + OFF, 8, 0, u, LO)
                cp(True, w * 8 + OFF, 8, 0, u, HI)
            else:
                cp(False, 24 + OFF, 8 - OFF, 0, u, LO)
                cp(True, 0, OFF, 8 - OFF, u, LO)
                cp(True, 24 + OFF, 8 - OFF, 0, u, HI)
                cp(False, 0, OFF, 8 - OFF, u, HI)
        go(ckv_hbm.at[w, rows(64 + p * 8 + j, 32)], c_v.at[s, rows(8 + j, 32)], S_C + s, LO)
        go(ckv_hbm.at[w, rows(p * 8 + j, 32)], c_v.at[s, rows(j, 32)], S_C + s, HI)

    def issue_unit(i, wrap):
        loop(0, 7, lambda j: tick_main(i, j, wrap))
        tick_main(i, 7, wrap)

    def tick_e(t):
        fin = t >= 112
        q = jnp.where(fin, (t >> 2) & 3, t & 3)
        r = rows(jnp.where(fin, 28 + (t & 3), t >> 2), 32)
        go(woa_hbm.at[q, r], woa_v.at[q, r], S_WOA + jnp.where(fin, 7 + q, t >> 4), LO)
        go(wob_hbm.at[:, rows(t, 8)], wob_v.at[:, rows(t, 8)], S_WOB + (t >> 4), HI)

    tick_pa(0, LO)
    cxa = pltpu.make_async_copy(xa_hbm, xa_v, sem.at[S_X])
    cxb = pltpu.make_async_copy(xb_hbm, xb_v, sem.at[S_X + 1])
    cxa.start()
    cxb.start()
    loop(1, PRE, lambda t: tick_pa(t, LO))
    loop(PRE, 64, tick_pa)

    cxa.wait()
    cxb.wait()
    ex = (_iota((128, 256), 1) // 2 == _iota((128, 256), 0)).astype(BF16)
    par8 = (_iota((8, 256), 1) % 2) == (_iota((8, 256), 0) // 4)
    xa = xa_v[...].astype(F32)
    xa8 = jnp.concatenate([xa, xa], axis=0).astype(BF16)
    for n in range(4):
        t = jnp.where(par8, _dot(xa8[:, n * 128:(n + 1) * 128], ex), 0.0)
        x2_s[2 * n] = t[:, :128]
        x2_s[2 * n + 1] = t[:, 128:]

    def init(b):
        ma_s[b] = jnp.full(ma_s.shape[1:], -jnp.inf, F32)
        la_s[b] = jnp.zeros(la_s.shape[1:], F32)
        acca_s[b] = jnp.zeros(acca_s.shape[1:], F32)
        mb_s[b] = jnp.full(mb_s.shape[1:], -jnp.inf, F32)
        lb_s[b] = jnp.zeros(lb_s.shape[1:], F32)
        accb_s[b] = jnp.zeros(accb_s.shape[1:], F32)
        qb_s[rows(32 + b, 8), :] = jnp.zeros((8, 128), F32)
        og_s[rows(4 + b, 64), :] = jnp.zeros((64, 128), F32)
    loop(0, B, init)

    loop(64, 128, tick_pa)
    loop(0, 40, tick_pb)

    wait_all(wqb_v, S_WQB)
    xb = xb_v[...].astype(F32)
    xb8 = jnp.concatenate([xb, xb], axis=0).astype(BF16)

    def qb_job(j):
        loop(40 + 4 * j, 44 + 4 * j, tick_pb)
        q = _dot(xb8, wqb_v[:, :, rows(j, 512)].reshape(M, 512))
        for u in range(4):
            qb_s[rows(4 * j + u, 8), :] = q[:, u * 128:(u + 1) * 128]
    loop(0, 8, qb_job)
    for w in range(4):
        for r in range(8):
            g = (8 * w + OFF + r) % 32
            qg_s[w, pl.ds(r * 8, 8), :] = qb_s[pl.ds((g % 8) * 32 + g // 8, 8, stride=8), :]
    loop(72, 128, tick_pb)
    loop(0, 8, lambda j: tick_main(0, j))

    def stage(w_v, j):
        w32_s[...] = pltpu.bitcast(w_v[j], jnp.uint32)

    def tile(p):
        return pltpu.bitcast(w32_s[pl.ds(p, 64, stride=16), :], BF16)

    wait_all(wqa_v, S_WQA)

    def qa_job(j, acc):
        tick_main(1, j)
        stage(wqa_v, j)
        w = jnp.concatenate([tile(p) for p in range(16)], axis=1)
        return acc + _dot(x2_s[j].astype(BF16), w)
    qa = lax.fori_loop(0, 8, qa_job, jnp.zeros((8, 2048), F32)).astype(BF16)

    wait_all(wuk_v, S_WUK)
    parw = (_iota((128, 128), 1) % 2) == ((_iota((128, 128), 0) // 4) % 2)

    def qabs_job(j):
        tick_main(2, j)
        stage(wuk_v, j)
        r = [_dot(qa[:, p * 128:(p + 1) * 128], tile(p), NT) for p in range(16)]
        r_s[j] = jnp.where(parw, jnp.concatenate(r, axis=0), 0.0).astype(BF16)
    loop(0, 8, qabs_job)

    cmp = (_iota((256, 128), 0) // 2 == _iota((256, 128), 1)).astype(BF16)
    perm = ((_iota((128, 128), 0) % 32) * 4 + _iota((128, 128), 0) // 32
            == _iota((128, 128), 1)).astype(BF16)

    def pack_job(n):
        t = _dot(jnp.concatenate([r_s[2 * n], r_s[2 * n + 1]], axis=1), cmp).astype(BF16)
        qabs_s[n] = _dot(perm, t).astype(BF16)
    loop(0, 4, pack_job)

    def online(sc, m_s, l_s, b):
        sc = (sc.astype(BF16).astype(F32) * SCALE).astype(BF16).astype(F32)
        m_old = m_s[b]
        m_new = jnp.maximum(m_old, jnp.max(sc, axis=-1, keepdims=True))
        alpha = jnp.exp(m_old - m_new)
        p = jnp.exp(sc - jnp.tile(m_new, (1, 4)))
        l_s[b] = alpha * l_s[b] + ((p[:, 0:128] + p[:, 128:256]) + (p[:, 256:384] + p[:, 384:512]))
        m_s[b] = m_new
        return p, alpha

    def main(i):
        @pl.when(i < 24 - LAG)
        def _():
            issue_unit(i + LAG, False)

        @pl.when(jnp.logical_and(i >= 24 - LAG, i < NIT - LAG))
        def _():
            issue_unit(i + LAG, True)

        @pl.when(i >= NIT - LAG)
        def _():
            e = i - (NIT - LAG)
            loop(e * 18, e * 18 + 18, tick_e)

        @pl.when(i < 8)
        def _():
            stage(wuv_v, i)
            for p in range(16):
                wuv_v[i, pl.ds(p * 128, 128), :] = tile(p)

        s, b = i & (RING - 1), i >> 3
        wait_all(k_v.at[s], S_K + s)
        wait_all(v_v.at[s], S_V + s)
        wait_all(c_v.at[s], S_C + s)
        sc = [_dot(qg_s[b, pl.ds(g * 8, 8), :].astype(BF16), k_v[s, g], NT) for g in range(HKV)]
        p, alpha = online(jnp.concatenate(sc, axis=0), mb_s, lb_s, b)

        q = jnp.concatenate([qabs_s[n, rows(b, 32), :] for n in range(4)], axis=1)
        pa, alpha_a = online(_dot(q, c_v[s], NT), ma_s, la_s, b)

        o = [_dot(p[g * 8:(g + 1) * 8].astype(BF16), v_v[s, g]) for g in range(HKV)]
        accb_s[b] = accb_s[b] * alpha + jnp.concatenate(o, axis=0)
        acca_s[b] = acca_s[b] * jnp.tile(alpha_a, (1, 4)) + _dot(pa.astype(BF16), c_v[s])

    wait_all(wuv_v, S_WUV)
    loop(0, NIT, main)

    for b in range(B):
        o = accb_s[b] / jnp.sum(lb_s[b], axis=-1, keepdims=True)
        if b < 3:
            og_s[pl.ds(b * 64 + OFF * 8, 64), :] = o
        else:
            og_s[pl.ds(192 + OFF * 8, 64 - OFF * 8), :] = o[:64 - OFF * 8]
            og_s[pl.ds(0, OFF * 8), :] = o[64 - OFF * 8:]
        acca_s[b] = acca_s[b] / jnp.sum(la_s[b], axis=-1, keepdims=True)
    for h in range(H):
        ob_s[h % 8, :, pl.ds((h // 8) * 128, 128)] = (
            og_s[pl.ds((h // 4) * 8 + h % 4, 8, stride=64), :])

    permt = ((_iota((128, 128), 1) % 32) * 4 + _iota((128, 128), 1) // 32
             == _iota((128, 128), 0)).astype(BF16)
    par128 = (_iota((128, 256), 1) % 2) == ((_iota((128, 256), 0) // 4) % 2)

    def expand_job(n):
        loop(54 + n * 4, 58 + n * 4, tick_e)
        cc = acca_s[:, :, rows(n, 128)].reshape(128, 128).astype(BF16)
        t = jnp.where(par128, _dot(_dot(permt, cc).astype(BF16), ex), 0.0)
        lx_s[2 * n] = t[:, :128]
        lx_s[2 * n + 1] = t[:, 128:]
    loop(0, 4, expand_job)

    def ctx_job(j, acc):
        loop(70 + 2 * j, 72 + 2 * j, tick_e)
        return acc + jnp.concatenate(
            [_dot(lx_s[j, pl.ds(p * 8, 8), :].astype(BF16), wuv_v[j, pl.ds(p * 128, 128), :])
             for p in range(16)], axis=0)
    ctx = lax.fori_loop(0, 8, ctx_job, jnp.zeros((128, 128), F32))
    top = _iota((8, 128), 0) < 4
    for h in range(H):
        c = ctx[(h // 2) * 8:(h // 2) * 8 + 8]
        if h % 8 == 7:
            c = jnp.concatenate([c[4:], c[:4]], axis=0)
        else:
            c = jnp.where(top, c, 0.0) if h % 2 == 0 else jnp.where(top, 0.0, c)
        lo_s[h % 8, :, pl.ds((h // 8) * 128, 128)] = c

    def proj(lhs_s, w_v, a, s):
        blk = w_v.at[:, rows(a, 128)]
        lhs = lhs_s[a].astype(BF16)
        wait_all(blk, s)
        return _dot(lhs, blk[...].reshape(512, M))

    def wo_job(a, carry):
        outa, outb = carry
        loop(jnp.minimum(86 + 11 * a, 128), jnp.minimum(97 + 11 * a, 128), tick_e)
        outb = outb + proj(ob_s, wob_v, a + 1, S_WOB + a + 1)
        outa = outa + proj(lo_s, woa_v, a, S_WOA + a)
        return outa, outb
    outa, outb = lax.fori_loop(0, 7, wo_job, (jnp.zeros((8, M), F32), proj(ob_s, wob_v, 0, S_WOB)))
    o_v[:, M:] = outb[0:4].astype(BF16)
    outa = outa + jnp.concatenate([outa[4:], outa[:4]], axis=0)

    def fin_job(q, acc):
        blk = woa_v.at[q, pl.ds(896, 128)]
        lhs = lo_s[7, :, rows(q, 128)].astype(BF16)
        wait_all(blk, S_WOA + 7 + q)
        return acc + _dot(lhs, blk[...])
    outa = lax.fori_loop(0, 4, fin_job, outa)
    o_v[:, :M] = outa[0:4].astype(BF16)
    co = pltpu.make_async_copy(o_v, o_hbm, sem.at[S_X])
    co.start()
    co.wait()


@jax.jit
def pallas_concat_heads__compressed_kv_cla__gqa_block_cached__decode_kernel(
    A_x: jax.Array,
    A_c_kv: jax.Array,
    A_w_q: jax.Array,
    A_w_uk: jax.Array,
    A_w_uv: jax.Array,
    A_w_o: jax.Array,
    B_x: jax.Array,
    B_k_cache: jax.Array,
    B_v_cache: jax.Array,
    B_wq: jax.Array,
    B_wo: jax.Array,
):
    args = (
        A_x.reshape(B, M),
        A_c_kv,
        A_w_q.reshape(8, 2048, D),
        A_w_uk.reshape(8, 2048, D),
        A_w_uv.reshape(8, 2048, D),
        A_w_o.reshape(4, 1024, M),
        B_x.reshape(B, M),
        B_k_cache.reshape(B * HKV, S, D),
        B_v_cache.reshape(B * HKV, S, D),
        B_wq.reshape(8, 64, H * D),
        B_wo.reshape(4, 1024, M),
    )
    V = pltpu.VMEM
    scratch = [
        V((B, M), BF16), V((B, M), BF16), V((B, 2 * M), BF16),
        V((RING, HKV, 512, D), BF16), V((RING, HKV, 512, D), BF16), V((RING, 512, DC), BF16),
        V((8, 2048, D), BF16), V((8, 2048, D), BF16), V((8, 2048, D), BF16),
        V((8, 64, H * D), BF16), V((4, 1024, M), BF16), V((4, 1024, M), BF16),
        V((8, 8, 128), F32),
        V((8, 128, 128), BF16),
        V((4, 128, 128), BF16),
        V((256 + 32, D), F32),
        V((B, 64, D), F32),
        V((512, D), F32),
        V((8, 8, 512), F32),
        V((B, H, 128), F32), V((B, H, 128), F32), V((B, H, DC), F32),
        V((B, 64, 128), F32), V((B, 64, 128), F32), V((B, 64, D), F32),
        V((8, 128, 128), F32),
        V((8, 8, 512), F32),
        V((1024, 128), jnp.uint32),
        pltpu.SemaphoreType.DMA((S_N,)),
    ]
    out = pl.pallas_call(
        _kernel,
        in_specs=[pl.BlockSpec(memory_space=pl.ANY)] * 11,
        out_specs=pl.BlockSpec(memory_space=pl.ANY),
        out_shape=jax.ShapeDtypeStruct((B, 2 * M), BF16),
        scratch_shapes=scratch,
        compiler_params=pltpu.CompilerParams(
            vmem_limit_bytes=64 * 1024 * 1024,
            disable_bounds_checks=True,
            disable_semaphore_checks=True,
        ),
    )(*args)
    return out.reshape(B, 1, 2 * M)
```

```python
import jax
import jax.numpy as jnp
from jax import lax
import jax.experimental.pallas as pl
import jax.experimental.pallas.tpu as pltpu

F32 = jnp.float32
BF16 = jnp.bfloat16
NT = (((1,), (1,)), ((), ()))
NN = (((1,), (0,)), ((), ()))

B = 4
H = 32
D = 128
M = 512
DC = 512
S = 4096
HKV = 8
NIT = 32
RING = 4
LAG = 3
OFF = 2
SH = 8
HI, LO = 0, 1
PRE = 7
SCALE = 0.08837890625

S_K, S_V, S_C, S_WQA, S_WUK, S_WQB, S_WUV, S_X, S_WOB, S_WOA, S_N = (
    0, 4, 8, 12, 13, 14, 15, 16, 18, 26, 37)


def _dot(a, b, dims=NN):
    return lax.dot_general(a, b, dims, preferred_element_type=F32)


def _iota(shape, dim):
    return lax.broadcasted_iota(jnp.int32, shape, dim)


def _kernel(xa_hbm, ckv_hbm, wqa_hbm, wuk_hbm, wuv_hbm, woa_hbm,
            xb_hbm, k_hbm, v_hbm, wqb_hbm, wob_hbm,
            o_hbm,
            xa_v, xb_v, o_v, k_v, v_v, c_v, wqa_v, wuk_v, wuv_v, wqb_v, woa_v, wob_v,
            x2_s, r_s, qabs_s, qb_s, qg_s, og_s, ob_s,
            ma_s, la_s, acca_s, mb_s, lb_s, accb_s, lx_s, lo_s, w32_s, sem):

    def ds(start, n, align):
        if isinstance(start, int):
            return pl.ds(start, n)
        return pl.ds(pl.multiple_of(start, align), n)

    def rows(i, n):
        return ds(i * n, n, n)

    def go(src, dst, s, prio):
        pltpu.make_async_copy(src, dst, sem.at[s]).start(priority=prio)

    def wait_all(buf, s):
        pltpu.make_async_copy(buf, buf, sem.at[s]).wait()

    def loop(lo, hi, fn):
        def body(i, c):
            fn(i)
            return c
        lax.fori_loop(lo, hi, body, 0)

    def cp_n(src, dst, half, t, s, prio):
        g = pl.ds(half * 4, 4)
        go(src.at[g, rows(t, 16)], dst.at[g, rows(t, 16)], s, prio)

    def cp_q(half, t, prio):
        g, r, c = pl.ds(half * 4, 4), rows(t >> 4, 8), rows(t & 15, 256)
        go(wqb_hbm.at[g, r, c], wqb_v.at[g, r, c], S_WQB, prio)

    def tick_pa(t, hi=HI):
        cp_n(wqa_hbm, wqa_v, 1, t, S_WQA, LO)
        cp_q(0, t, LO)
        cp_n(wuv_hbm, wuv_v, 0, t, S_WUV, hi)
        cp_q(1, t, hi)

    def tick_pb(t):
        cp_n(wuk_hbm, wuk_v, 0, t, S_WUK, LO)
        cp_n(wuv_hbm, wuv_v, 1, t, S_WUV, LO)
        cp_n(wqa_hbm, wqa_v, 0, t, S_WQA, HI)
        cp_n(wuk_hbm, wuk_v, 1, t, S_WUK, HI)

    def tick_main(i, j, wrap=False):
        s, w, p = i & (RING - 1), i >> 3, i & 7

        def cp(is_k, g0, n, d0, u, prio):
            src, dst, sm = (k_hbm, k_v, S_K) if is_k else (v_hbm, v_v, S_V)
            a = j * 64 + u * 16
            segs = [(p * 512 + a + SH, a, 16)]
            if isinstance(j, int) and a == 496:
                segs = [(p * 512 + a + SH, a, 16 - SH), ((p * 512 + 512) & (S - 1), 512 - SH, SH)]
            for rs, rd, nr in segs:
                go(src.at[pl.ds(g0, n), ds(rs, nr, 8)], dst.at[s, pl.ds(d0, n), ds(rd, nr, 8)],
                   sm + s, prio)

        for u in range(4):
            if not wrap:
                cp(False, w * 8 + OFF, 8, 0, u, LO)
                cp(True, w * 8 + OFF, 8, 0, u, HI)
            else:
                cp(False, 24 + OFF, 8 - OFF, 0, u, LO)
                cp(True, 0, OFF, 8 - OFF, u, LO)
                cp(True, 24 + OFF, 8 - OFF, 0, u, HI)
                cp(False, 0, OFF, 8 - OFF, u, HI)
        go(ckv_hbm.at[w, rows(64 + p * 8 + j, 32)], c_v.at[s, rows(8 + j, 32)], S_C + s, LO)
        go(ckv_hbm.at[w, rows(p * 8 + j, 32)], c_v.at[s, rows(j, 32)], S_C + s, HI)

    def issue_unit(i, wrap):
        loop(0, 7, lambda j: tick_main(i, j, wrap))
        tick_main(i, 7, wrap)

    def tick_e(t):
        fin = t >= 112
        q = jnp.where(fin, (t >> 2) & 3, t & 3)
        r = rows(jnp.where(fin, 28 + (t & 3), t >> 2), 32)
        go(woa_hbm.at[q, r], woa_v.at[q, r], S_WOA + jnp.where(fin, 7 + q, t >> 4), LO)
        go(wob_hbm.at[:, rows(t, 8)], wob_v.at[:, rows(t, 8)], S_WOB + (t >> 4), HI)

    tick_pa(0, LO)
    cxa = pltpu.make_async_copy(xa_hbm, xa_v, sem.at[S_X])
    cxb = pltpu.make_async_copy(xb_hbm, xb_v, sem.at[S_X + 1])
    cxa.start()
    cxb.start()
    loop(1, PRE, lambda t: tick_pa(t, LO))
    loop(PRE, 64, tick_pa)

    cxa.wait()
    cxb.wait()
    ex = (_iota((128, 256), 1) // 2 == _iota((128, 256), 0)).astype(BF16)
    par8 = (_iota((8, 256), 1) % 2) == (_iota((8, 256), 0) // 4)
    xa = xa_v[...].astype(F32)
    xa8 = jnp.concatenate([xa, xa], axis=0).astype(BF16)
    for n in range(4):
        t = jnp.where(par8, _dot(xa8[:, n * 128:(n + 1) * 128], ex), 0.0)
        x2_s[2 * n] = t[:, :128]
        x2_s[2 * n + 1] = t[:, 128:]

    def init(b):
        ma_s[b] = jnp.full(ma_s.shape[1:], -jnp.inf, F32)
        la_s[b] = jnp.zeros(la_s.shape[1:], F32)
        acca_s[b] = jnp.zeros(acca_s.shape[1:], F32)
        mb_s[b] = jnp.full(mb_s.shape[1:], -jnp.inf, F32)
        lb_s[b] = jnp.zeros(lb_s.shape[1:], F32)
        accb_s[b] = jnp.zeros(accb_s.shape[1:], F32)
        qb_s[rows(32 + b, 8), :] = jnp.zeros((8, 128), F32)
        og_s[rows(4 + b, 64), :] = jnp.zeros((64, 128), F32)
    loop(0, B, init)

    loop(64, 128, tick_pa)
    loop(0, 40, tick_pb)

    wait_all(wqb_v, S_WQB)
    xb = xb_v[...].astype(F32)
    xb8 = jnp.concatenate([xb, xb], axis=0).astype(BF16)

    def qb_job(j):
        loop(0, 4, lambda u: tick_pb(40 + 4 * j + u))
        q = _dot(xb8, wqb_v[:, :, rows(j, 512)].reshape(M, 512))
        for u in range(4):
            qb_s[rows(4 * j + u, 8), :] = q[:, u * 128:(u + 1) * 128]
    loop(0, 8, qb_job)
    for w in range(4):
        for r in range(8):
            g = (8 * w + OFF + r) % 32
            qg_s[w, pl.ds(r * 8, 8), :] = qb_s[pl.ds((g % 8) * 32 + g // 8, 8, stride=8), :]
    loop(72, 128, tick_pb)
    loop(0, 8, lambda j: tick_main(0, j))

    def stage(w_v, j):
        w32_s[...] = pltpu.bitcast(w_v[j], jnp.uint32)

    def tile(p):
        return pltpu.bitcast(w32_s[pl.ds(p, 64, stride=16), :], BF16)

    wait_all(wqa_v, S_WQA)

    def qa_job(j, acc):
        tick_main(1, j)
        stage(wqa_v, j)
        w = jnp.concatenate([tile(p) for p in range(16)], axis=1)
        return acc + _dot(x2_s[j].astype(BF16), w)
    qa = lax.fori_loop(0, 8, qa_job, jnp.zeros((8, 2048), F32)).astype(BF16)

    wait_all(wuk_v, S_WUK)
    parw = (_iota((128, 128), 1) % 2) == ((_iota((128, 128), 0) // 4) % 2)

    def qabs_job(j):
        tick_main(2, j)
        stage(wuk_v, j)
        r = [_dot(qa[:, p * 128:(p + 1) * 128], tile(p), NT) for p in range(16)]
        r_s[j] = jnp.where(parw, jnp.concatenate(r, axis=0), 0.0).astype(BF16)
    loop(0, 8, qabs_job)

    cmp = (_iota((256, 128), 0) // 2 == _iota((256, 128), 1)).astype(BF16)
    perm = ((_iota((128, 128), 0) % 32) * 4 + _iota((128, 128), 0) // 32
            == _iota((128, 128), 1)).astype(BF16)

    def pack_job(n):
        t = _dot(jnp.concatenate([r_s[2 * n], r_s[2 * n + 1]], axis=1), cmp).astype(BF16)
        qabs_s[n] = _dot(perm, t).astype(BF16)
    loop(0, 4, pack_job)

    def online(sc, m_s, l_s, b):
        sc = (sc.astype(BF16).astype(F32) * SCALE).astype(BF16).astype(F32)
        m_old = m_s[b]
        m_new = jnp.maximum(m_old, jnp.max(sc, axis=-1, keepdims=True))
        alpha = jnp.exp(m_old - m_new)
        p = jnp.exp(sc - jnp.tile(m_new, (1, 4)))
        l_s[b] = alpha * l_s[b] + ((p[:, 0:128] + p[:, 128:256]) + (p[:, 256:384] + p[:, 384:512]))
        m_s[b] = m_new
        return p, alpha

    def main(i):
        @pl.when(i < 24 - LAG)
        def _():
            issue_unit(i + LAG, False)

        @pl.when(jnp.logical_and(i >= 24 - LAG, i < NIT - LAG))
        def _():
            issue_unit(i + LAG, True)

        @pl.when(i >= NIT - LAG)
        def _():
            loop(0, 24, lambda u: tick_e((i - (NIT - LAG)) * 24 + u))

        @pl.when(i < 8)
        def _():
            stage(wuv_v, i)
            for p in range(16):
                wuv_v[i, pl.ds(p * 128, 128), :] = tile(p)

        s, b = i & (RING - 1), i >> 3
        wait_all(k_v.at[s], S_K + s)
        wait_all(v_v.at[s], S_V + s)
        wait_all(c_v.at[s], S_C + s)
        sc = [_dot(qg_s[b, pl.ds(g * 8, 8), :].astype(BF16), k_v[s, g], NT) for g in range(HKV)]
        p, alpha = online(jnp.concatenate(sc, axis=0), mb_s, lb_s, b)

        q = jnp.concatenate([qabs_s[n, rows(b, 32), :] for n in range(4)], axis=1)
        pa, alpha_a = online(_dot(q, c_v[s], NT), ma_s, la_s, b)

        o = [_dot(p[g * 8:(g + 1) * 8].astype(BF16), v_v[s, g]) for g in range(HKV)]
        accb_s[b] = accb_s[b] * alpha + jnp.concatenate(o, axis=0)
        acca_s[b] = acca_s[b] * jnp.tile(alpha_a, (1, 4)) + _dot(pa.astype(BF16), c_v[s])

    wait_all(wuv_v, S_WUV)
    loop(0, NIT, main)

    for b in range(B):
        o = accb_s[b] / jnp.sum(lb_s[b], axis=-1, keepdims=True)
        if b < 3:
            og_s[pl.ds(b * 64 + OFF * 8, 64), :] = o
        else:
            og_s[pl.ds(192 + OFF * 8, 64 - OFF * 8), :] = o[:64 - OFF * 8]
            og_s[pl.ds(0, OFF * 8), :] = o[64 - OFF * 8:]
        acca_s[b] = acca_s[b] / jnp.sum(la_s[b], axis=-1, keepdims=True)
    for h in range(H):
        ob_s[h % 8, :, pl.ds((h // 8) * 128, 128)] = (
            og_s[pl.ds((h // 4) * 8 + h % 4, 8, stride=64), :])

    permt = ((_iota((128, 128), 1) % 32) * 4 + _iota((128, 128), 1) // 32
             == _iota((128, 128), 0)).astype(BF16)
    par128 = (_iota((128, 256), 1) % 2) == ((_iota((128, 256), 0) // 4) % 2)

    def expand_job(n):
        loop(0, 6, lambda u: tick_e(72 + 6 * n + u))
        cc = acca_s[:, :, rows(n, 128)].reshape(128, 128).astype(BF16)
        t = jnp.where(par128, _dot(_dot(permt, cc).astype(BF16), ex), 0.0)
        lx_s[2 * n] = t[:, :128]
        lx_s[2 * n + 1] = t[:, 128:]
    loop(0, 4, expand_job)

    def ctx_job(j, acc):
        loop(0, 4, lambda u: tick_e(96 + 4 * j + u))
        return acc + jnp.concatenate(
            [_dot(lx_s[j, pl.ds(p * 8, 8), :].astype(BF16), wuv_v[j, pl.ds(p * 128, 128), :])
             for p in range(16)], axis=0)
    ctx = lax.fori_loop(0, 8, ctx_job, jnp.zeros((128, 128), F32))
    top = _iota((8, 128), 0) < 4
    for h in range(H):
        c = ctx[(h // 2) * 8:(h // 2) * 8 + 8]
        if h % 8 == 7:
            c = jnp.concatenate([c[4:], c[:4]], axis=0)
        else:
            c = jnp.where(top, c, 0.0) if h % 2 == 0 else jnp.where(top, 0.0, c)
        lo_s[h % 8, :, pl.ds((h // 8) * 128, 128)] = c

    def arrive(w_v, a, s):
        wait_all(w_v.at[:, rows(a, 128)], s + a)

    def proj(lhs_s, w_v, a):
        return _dot(lhs_s[a].astype(BF16), w_v[:, rows(a, 128), :].reshape(512, M))

    def wo_job(a, carry):
        arrive(wob_v, a + 1, S_WOB)
        arrive(woa_v, a, S_WOA)
        return carry[0] + proj(lo_s, woa_v, a), carry[1] + proj(ob_s, wob_v, a + 1)
    arrive(wob_v, 0, S_WOB)
    outa, outb = lax.fori_loop(0, 6, wo_job, (jnp.zeros((8, M), F32), proj(ob_s, wob_v, 0)))
    arrive(wob_v, 7, S_WOB)
    outb = outb + proj(ob_s, wob_v, 7)
    arrive(woa_v, 6, S_WOA)
    outa = outa + proj(lo_s, woa_v, 6)
    o_v[:, M:] = outb[0:4].astype(BF16)
    outa = outa + jnp.concatenate([outa[4:], outa[:4]], axis=0)

    def fin_job(q, acc):
        blk = woa_v.at[q, pl.ds(896, 128)]
        lhs = lo_s[7, :, rows(q, 128)].astype(BF16)
        wait_all(blk, S_WOA + 7 + q)
        return acc + _dot(lhs, blk[...])
    outa = lax.fori_loop(0, 4, fin_job, outa)
    o_v[:, :M] = outa[0:4].astype(BF16)
    co = pltpu.make_async_copy(o_v, o_hbm, sem.at[S_X])
    co.start()
    co.wait()


@jax.jit
def pallas_concat_heads__compressed_kv_cla__gqa_block_cached__decode_kernel(
    A_x: jax.Array,
    A_c_kv: jax.Array,
    A_w_q: jax.Array,
    A_w_uk: jax.Array,
    A_w_uv: jax.Array,
    A_w_o: jax.Array,
    B_x: jax.Array,
    B_k_cache: jax.Array,
    B_v_cache: jax.Array,
    B_wq: jax.Array,
    B_wo: jax.Array,
):
    args = (
        A_x.reshape(B, M),
        A_c_kv,
        A_w_q.reshape(8, 2048, D),
        A_w_uk.reshape(8, 2048, D),
        A_w_uv.reshape(8, 2048, D),
        A_w_o.reshape(4, 1024, M),
        B_x.reshape(B, M),
        B_k_cache.reshape(B * HKV, S, D),
        B_v_cache.reshape(B * HKV, S, D),
        B_wq.reshape(8, 64, H * D),
        B_wo.reshape(4, 1024, M),
    )
    V = pltpu.VMEM
    scratch = [
        V((B, M), BF16), V((B, M), BF16), V((B, 2 * M), BF16),
        V((RING, HKV, 512, D), BF16), V((RING, HKV, 512, D), BF16), V((RING, 512, DC), BF16),
        V((8, 2048, D), BF16), V((8, 2048, D), BF16), V((8, 2048, D), BF16),
        V((8, 64, H * D), BF16), V((4, 1024, M), BF16), V((4, 1024, M), BF16),
        V((8, 8, 128), F32),
        V((8, 128, 128), BF16),
        V((4, 128, 128), BF16),
        V((256 + 32, D), F32),
        V((B, 64, D), F32),
        V((512, D), F32),
        V((8, 8, 512), F32),
        V((B, H, 128), F32), V((B, H, 128), F32), V((B, H, DC), F32),
        V((B, 64, 128), F32), V((B, 64, 128), F32), V((B, 64, D), F32),
        V((8, 128, 128), F32),
        V((8, 8, 512), F32),
        V((1024, 128), jnp.uint32),
        pltpu.SemaphoreType.DMA((S_N,)),
    ]
    out = pl.pallas_call(
        _kernel,
        in_specs=[pl.BlockSpec(memory_space=pl.ANY)] * 11,
        out_specs=pl.BlockSpec(memory_space=pl.ANY),
        out_shape=jax.ShapeDtypeStruct((B, 2 * M), BF16),
        scratch_shapes=scratch,
        compiler_params=pltpu.CompilerParams(
            vmem_limit_bytes=64 * 1024 * 1024,
            disable_bounds_checks=True,
            disable_semaphore_checks=True,
        ),
    )(*args)
    return out.reshape(B, 1, 2 * M)
```

```python
import jax
import jax.numpy as jnp
from jax import lax
import jax.experimental.pallas as pl
import jax.experimental.pallas.tpu as pltpu

F32 = jnp.float32
BF16 = jnp.bfloat16
NT = (((1,), (1,)), ((), ()))
NN = (((1,), (0,)), ((), ()))

B = 4
H = 32
D = 128
M = 512
DC = 512
S = 4096
HKV = 8
NIT = 32
RING = 4
LAG = 2
OFF = 2
SH = 8
HI, LO = 0, 1
PRE = 4
SCALE = 0.08837890625

S_K, S_V, S_C, S_WQA, S_WUK, S_WQB, S_WUV, S_X, S_WOB, S_WOA, S_FIN, S_N = (
    0, 4, 8, 12, 13, 14, 15, 16, 18, 26, 34, 38)


def _dot(a, b, dims=NN):
    return lax.dot_general(a, b, dims, preferred_element_type=F32)


def _iota(shape, dim):
    return lax.broadcasted_iota(jnp.int32, shape, dim)


def _kernel(xa_hbm, ckv_hbm, wqa_hbm, wuk_hbm, wuv_hbm, woa_hbm,
            xb_hbm, k_hbm, v_hbm, wqb_hbm, wob_hbm,
            o_hbm,
            xa_v, xb_v, o_v, k_v, v_v, c_v, wqa_v, wuk_v, wuv_v, wqb_v, woa_v, wob_v,
            x2_s, r_s, qabs_s, qb_s, qg_s, og_s, ob_s,
            ma_s, la_s, acca_s, mb_s, lb_s, accb_s, lx_s, lo_s, w32_s, sem):

    def ds(start, n, align):
        if isinstance(start, int):
            return pl.ds(start, n)
        return pl.ds(pl.multiple_of(start, align), n)

    def rows(i, n):
        return ds(i * n, n, n)

    def go(src, dst, s, prio):
        pltpu.make_async_copy(src, dst, sem.at[s]).start(priority=prio)

    def wait_all(buf, s):
        pltpu.make_async_copy(buf, buf, sem.at[s]).wait()

    def loop(lo, hi, fn):
        def body(i, c):
            fn(i)
            return c
        lax.fori_loop(lo, hi, body, 0)

    def cp_n(src, dst, half, t, s, prio):
        g = pl.ds(half * 4, 4)
        go(src.at[g, rows(t, 16)], dst.at[g, rows(t, 16)], s, prio)

    def cp_q(half, t, prio):
        g, r, c = pl.ds(half * 4, 4), rows(t >> 4, 8), rows(t & 15, 256)
        go(wqb_hbm.at[g, r, c], wqb_v.at[g, r, c], S_WQB, prio)

    def tick_p1(t, hi=HI):
        for u in range(2):
            cp_n(wqa_hbm, wqa_v, 1, 2 * t + u, S_WQA, LO)
            cp_q(0, 2 * t + u, LO)
        cp_q(1, t, hi)

    def tick_p2(t):
        for u in range(2):
            cp_n(wqa_hbm, wqa_v, 0, 2 * t + u, S_WQA, LO)
            cp_n(wuk_hbm, wuk_v, 1, 2 * t + u, S_WUK, LO)
        cp_q(1, 64 + t, HI)

    def tick_p3(t):
        cp_n(wuk_hbm, wuk_v, 0, t, S_WUK, LO)
        cp_n(wuv_hbm, wuv_v, 1, t, S_WUV, LO)
        cp_n(wuv_hbm, wuv_v, 0, t, S_WUV, HI)

    def tick_main(i, j, wrap=False):
        s, w, p = i & (RING - 1), i >> 3, i & 7

        def cp(is_k, g0, n, d0, u, prio):
            src, dst, sm = (k_hbm, k_v, S_K) if is_k else (v_hbm, v_v, S_V)
            a = j * 64 + u * 16
            segs = [(p * 512 + a + SH, a, 16)]
            if isinstance(j, int) and a == 496:
                segs = [(p * 512 + a + SH, a, 16 - SH), ((p * 512 + 512) & (S - 1), 512 - SH, SH)]
            for rs, rd, nr in segs:
                go(src.at[pl.ds(g0, n), ds(rs, nr, 8)], dst.at[s, pl.ds(d0, n), ds(rd, nr, 8)],
                   sm + s, prio)

        for u in range(4):
            if not wrap:
                cp(False, w * 8 + OFF, 8, 0, u, LO)
                cp(True, w * 8 + OFF, 8, 0, u, HI)
            else:
                cp(False, 24 + OFF, 8 - OFF, 0, u, LO)
                cp(True, 0, OFF, 8 - OFF, u, LO)
                cp(True, 24 + OFF, 8 - OFF, 0, u, HI)
                cp(False, 0, OFF, 8 - OFF, u, HI)
        go(ckv_hbm.at[w, rows(64 + p * 8 + j, 32)], c_v.at[s, rows(8 + j, 32)], S_C + s, LO)
        go(ckv_hbm.at[w, rows(p * 8 + j, 32)], c_v.at[s, rows(j, 32)], S_C + s, HI)

    def issue_unit(i, wrap):
        loop(0, 7, lambda j: tick_main(i, j, wrap))
        tick_main(i, 7, wrap)

    def tick_e(t, late):
        if not late:
            r = rows(t >> 2, 32)
            go(wob_hbm.at[4 + (t & 3), r], wob_v.at[4 + (t & 3), r], S_WOB + 4 + (t >> 4), LO)
        else:
            fin = t >= 112
            q = jnp.where(fin, (t >> 2) & 3, t & 3)
            r = rows(jnp.where(fin, 12 + (t & 3), (t >> 2) & 15), 32)
            go(woa_hbm.at[q, r], woa_v.at[q, r], jnp.where(fin, S_FIN + q, S_WOA - 4 + (t >> 4)), LO)
        r, c = rows(t >> 1, 8), rows(t & 1, 256)
        go(woa_hbm.at[pl.ds(4, 4), r, c], woa_v.at[pl.ds(4, 4), r, c], S_WOA + 4 + (t >> 5), HI)
        go(wob_hbm.at[pl.ds(0, 4), r, c], wob_v.at[pl.ds(0, 4), r, c], S_WOB + (t >> 5), HI)

    tick_p1(0, LO)
    cxa = pltpu.make_async_copy(xa_hbm, xa_v, sem.at[S_X])
    cxb = pltpu.make_async_copy(xb_hbm, xb_v, sem.at[S_X + 1])
    cxa.start()
    cxb.start()
    loop(1, PRE, lambda t: tick_p1(t, LO))
    loop(PRE, 64, tick_p1)

    cxa.wait()
    cxb.wait()
    ex = (_iota((128, 256), 1) // 2 == _iota((128, 256), 0)).astype(BF16)
    par8 = (_iota((8, 256), 1) % 2) == (_iota((8, 256), 0) // 4)
    xa = xa_v[...].astype(F32)
    xa8 = jnp.concatenate([xa, xa], axis=0).astype(BF16)
    for n in range(4):
        t = jnp.where(par8, _dot(xa8[:, n * 128:(n + 1) * 128], ex), 0.0)
        x2_s[2 * n] = t[:, :128]
        x2_s[2 * n + 1] = t[:, 128:]

    def init(b):
        ma_s[b] = jnp.full(ma_s.shape[1:], -jnp.inf, F32)
        la_s[b] = jnp.zeros(la_s.shape[1:], F32)
        acca_s[b] = jnp.zeros(acca_s.shape[1:], F32)
        mb_s[b] = jnp.full(mb_s.shape[1:], -jnp.inf, F32)
        lb_s[b] = jnp.zeros(lb_s.shape[1:], F32)
        accb_s[b] = jnp.zeros(accb_s.shape[1:], F32)
        qb_s[rows(32 + b, 8), :] = jnp.zeros((8, 128), F32)
        og_s[rows(4 + b, 64), :] = jnp.zeros((64, 128), F32)
    loop(0, B, init)

    loop(0, 64, tick_p2)
    loop(0, 32, tick_p3)

    wait_all(wqb_v, S_WQB)
    xb = xb_v[...].astype(F32)
    xb8 = jnp.concatenate([xb, xb], axis=0).astype(BF16)

    def qb_job(j):
        loop(0, 3, lambda u: tick_p3(32 + 3 * j + u))
        q = _dot(xb8, wqb_v[:, :, rows(j, 512)].reshape(M, 512))
        for u in range(4):
            qb_s[rows(4 * j + u, 8), :] = q[:, u * 128:(u + 1) * 128]
    loop(0, 8, qb_job)
    for w in range(4):
        for r in range(8):
            g = (8 * w + OFF + r) % 32
            qg_s[w, pl.ds(r * 8, 8), :] = qb_s[pl.ds((g % 8) * 32 + g // 8, 8, stride=8), :]

    def stage(w_v, j):
        w32_s[...] = pltpu.bitcast(w_v[j], jnp.uint32)

    def tile(p):
        return pltpu.bitcast(w32_s[pl.ds(p, 64, stride=16), :], BF16)

    wait_all(wqa_v, S_WQA)

    def qa_job(j, acc):
        loop(0, 6, lambda u: tick_p3(56 + 6 * j + u))
        stage(wqa_v, j)
        w = jnp.concatenate([tile(p) for p in range(16)], axis=1)
        return acc + _dot(x2_s[j].astype(BF16), w)
    qa = lax.fori_loop(0, 8, qa_job, jnp.zeros((8, 2048), F32)).astype(BF16)

    loop(104, 128, tick_p3)
    loop(0, 8, lambda j: tick_main(0, j))

    wait_all(wuk_v, S_WUK)
    parw = (_iota((128, 128), 1) % 2) == ((_iota((128, 128), 0) // 4) % 2)

    def qabs_job(j):
        tick_main(1, j)
        stage(wuk_v, j)
        r = [_dot(qa[:, p * 128:(p + 1) * 128], tile(p), NT) for p in range(16)]
        r_s[j] = jnp.where(parw, jnp.concatenate(r, axis=0), 0.0).astype(BF16)
    loop(0, 8, qabs_job)

    cmp = (_iota((256, 128), 0) // 2 == _iota((256, 128), 1)).astype(BF16)
    perm = ((_iota((128, 128), 0) % 32) * 4 + _iota((128, 128), 0) // 32
            == _iota((128, 128), 1)).astype(BF16)

    def pack_job(n):
        t = _dot(jnp.concatenate([r_s[2 * n], r_s[2 * n + 1]], axis=1), cmp).astype(BF16)
        qabs_s[n] = _dot(perm, t).astype(BF16)
    loop(0, 4, pack_job)

    def online(sc, m_s, l_s, b):
        sc = (sc.astype(BF16).astype(F32) * SCALE).astype(BF16).astype(F32)
        m_old = m_s[b]
        m_new = jnp.maximum(m_old, jnp.max(sc, axis=-1, keepdims=True))
        alpha = jnp.exp(m_old - m_new)
        p = jnp.exp(sc - jnp.tile(m_new, (1, 4)))
        l_s[b] = alpha * l_s[b] + ((p[:, 0:128] + p[:, 128:256]) + (p[:, 256:384] + p[:, 384:512]))
        m_s[b] = m_new
        return p, alpha

    def main(i):
        @pl.when(i < 24 - LAG)
        def _():
            issue_unit(i + LAG, False)

        @pl.when(jnp.logical_and(i >= 24 - LAG, i < NIT - LAG))
        def _():
            issue_unit(i + LAG, True)

        @pl.when(i >= NIT - LAG)
        def _():
            loop(0, 27, lambda u: tick_e((i - (NIT - LAG)) * 27 + u, False))

        @pl.when(i < 8)
        def _():
            stage(wuv_v, i)
            for p in range(16):
                wuv_v[i, pl.ds(p * 128, 128), :] = tile(p)

        s, b = i & (RING - 1), i >> 3
        wait_all(k_v.at[s], S_K + s)
        wait_all(v_v.at[s], S_V + s)
        wait_all(c_v.at[s], S_C + s)
        sc = [_dot(qg_s[b, pl.ds(g * 8, 8), :].astype(BF16), k_v[s, g], NT) for g in range(HKV)]
        p, alpha = online(jnp.concatenate(sc, axis=0), mb_s, lb_s, b)

        q = jnp.concatenate([qabs_s[n, rows(b, 32), :] for n in range(4)], axis=1)
        pa, alpha_a = online(_dot(q, c_v[s], NT), ma_s, la_s, b)

        o = [_dot(p[g * 8:(g + 1) * 8].astype(BF16), v_v[s, g]) for g in range(HKV)]
        accb_s[b] = accb_s[b] * alpha + jnp.concatenate(o, axis=0)
        acca_s[b] = acca_s[b] * jnp.tile(alpha_a, (1, 4)) + _dot(pa.astype(BF16), c_v[s])

    wait_all(wuv_v, S_WUV)
    loop(0, NIT, main)

    loop(54, 64, lambda t: tick_e(t, False))
    for b in range(B):
        o = accb_s[b] / jnp.sum(lb_s[b], axis=-1, keepdims=True)
        if b < 3:
            og_s[pl.ds(b * 64 + OFF * 8, 64), :] = o
        else:
            og_s[pl.ds(192 + OFF * 8, 64 - OFF * 8), :] = o[:64 - OFF * 8]
            og_s[pl.ds(0, OFF * 8), :] = o[64 - OFF * 8:]
        acca_s[b] = acca_s[b] / jnp.sum(la_s[b], axis=-1, keepdims=True)
    for h in range(H):
        ob_s[(h // 16) * 4 + h % 4, :, pl.ds((h // 4) % 4 * 128, 128)] = (
            og_s[pl.ds((h // 4) * 8 + h % 4, 8, stride=64), :])

    permt = ((_iota((128, 128), 1) % 32) * 4 + _iota((128, 128), 1) // 32
             == _iota((128, 128), 0)).astype(BF16)
    par128 = (_iota((128, 256), 1) % 2) == ((_iota((128, 256), 0) // 4) % 2)

    def expand_job(n):
        loop(0, 4, lambda u: tick_e(64 + 4 * n + u, True))
        cc = acca_s[:, :, rows(n, 128)].reshape(128, 128).astype(BF16)
        t = jnp.where(par128, _dot(_dot(permt, cc).astype(BF16), ex), 0.0)
        lx_s[2 * n] = t[:, :128]
        lx_s[2 * n + 1] = t[:, 128:]
    loop(0, 4, expand_job)

    def ctx_job(j, acc):
        loop(0, 3, lambda u: tick_e(80 + 3 * j + u, True))
        return acc + jnp.concatenate(
            [_dot(lx_s[j, pl.ds(p * 8, 8), :].astype(BF16), wuv_v[j, pl.ds(p * 128, 128), :])
             for p in range(16)], axis=0)
    ctx = lax.fori_loop(0, 8, ctx_job, jnp.zeros((128, 128), F32))
    top = _iota((8, 128), 0) < 4
    for h in range(H):
        c = ctx[(h // 2) * 8:(h // 2) * 8 + 8]
        if h < 16 and h % 4 == 3:
            c = jnp.concatenate([c[4:], c[:4]], axis=0)
        else:
            c = jnp.where(top, c, 0.0) if h % 2 == 0 else jnp.where(top, 0.0, c)
        lo_s[(h // 16) * 4 + h % 4, :, pl.ds((h // 4) % 4 * 128, 128)] = c

    def arrive(w_v, k, s):
        wait_all(w_v.at[pl.ds(k & 4, 4), rows(k & 3, 128)], s + k)

    def proj(lhs_s, w_v, k):
        w = w_v[pl.ds(k & 4, 4), rows(k & 3, 128), :]
        return _dot(lhs_s[k].astype(BF16), w.reshape(512, M))

    def wo_job(n, carry):
        @pl.when(n < 3)
        def _():
            loop(0, 8, lambda u: tick_e(104 + 8 * n + u, True))

        ka = (0x710654 >> (4 * n)) & 7
        kb = (0x327615 >> (4 * n)) & 7
        arrive(wob_v, kb, S_WOB)
        arrive(woa_v, ka, S_WOA)
        return carry[0] + proj(lo_s, woa_v, ka), carry[1] + proj(ob_s, wob_v, kb)
    arrive(wob_v, 0, S_WOB)
    arrive(wob_v, 4, S_WOB)
    outa, outb = lax.fori_loop(
        0, 6, wo_job, (jnp.zeros((8, M), F32), proj(ob_s, wob_v, 0) + proj(ob_s, wob_v, 4)))
    arrive(woa_v, 2, S_WOA)
    outa = outa + proj(lo_s, woa_v, 2)
    o_v[:, M:] = outb[0:4].astype(BF16)
    outa = outa + jnp.concatenate([outa[4:], outa[:4]], axis=0)

    def fin_job(q, acc):
        blk = woa_v.at[q, pl.ds(384, 128)]
        lhs = lo_s[3, :, rows(q, 128)].astype(BF16)
        wait_all(blk, S_FIN + q)
        return acc + _dot(lhs, blk[...])
    outa = lax.fori_loop(0, 4, fin_job, outa)
    o_v[:, :M] = outa[0:4].astype(BF16)
    co = pltpu.make_async_copy(o_v, o_hbm, sem.at[S_X])
    co.start()
    co.wait()


@jax.jit
def pallas_concat_heads__compressed_kv_cla__gqa_block_cached__decode_kernel(
    A_x: jax.Array,
    A_c_kv: jax.Array,
    A_w_q: jax.Array,
    A_w_uk: jax.Array,
    A_w_uv: jax.Array,
    A_w_o: jax.Array,
    B_x: jax.Array,
    B_k_cache: jax.Array,
    B_v_cache: jax.Array,
    B_wq: jax.Array,
    B_wo: jax.Array,
):
    args = (
        A_x.reshape(B, M),
        A_c_kv,
        A_w_q.reshape(8, 2048, D),
        A_w_uk.reshape(8, 2048, D),
        A_w_uv.reshape(8, 2048, D),
        A_w_o.reshape(8, 512, M),
        B_x.reshape(B, M),
        B_k_cache.reshape(B * HKV, S, D),
        B_v_cache.reshape(B * HKV, S, D),
        B_wq.reshape(8, 64, H * D),
        B_wo.reshape(8, 512, M),
    )
    V = pltpu.VMEM
    scratch = [
        V((B, M), BF16), V((B, M), BF16), V((B, 2 * M), BF16),
        V((RING, HKV, 512, D), BF16), V((RING, HKV, 512, D), BF16), V((RING, 512, DC), BF16),
        V((8, 2048, D), BF16), V((8, 2048, D), BF16), V((8, 2048, D), BF16),
        V((8, 64, H * D), BF16), V((8, 512, M), BF16), V((8, 512, M), BF16),
        V((8, 8, 128), F32),
        V((8, 128, 128), BF16),
        V((4, 128, 128), BF16),
        V((256 + 32, D), F32),
        V((B, 64, D), F32),
        V((512, D), F32),
        V((8, 8, 512), F32),
        V((B, H, 128), F32), V((B, H, 128), F32), V((B, H, DC), F32),
        V((B, 64, 128), F32), V((B, 64, 128), F32), V((B, 64, D), F32),
        V((8, 128, 128), F32),
        V((8, 8, 512), F32),
        V((1024, 128), jnp.uint32),
        pltpu.SemaphoreType.DMA((S_N,)),
    ]
    out = pl.pallas_call(
        _kernel,
        in_specs=[pl.BlockSpec(memory_space=pl.ANY)] * 11,
        out_specs=pl.BlockSpec(memory_space=pl.ANY),
        out_shape=jax.ShapeDtypeStruct((B, 2 * M), BF16),
        scratch_shapes=scratch,
        compiler_params=pltpu.CompilerParams(
            vmem_limit_bytes=64 * 1024 * 1024,
            disable_bounds_checks=True,
            disable_semaphore_checks=True,
        ),
    )(*args)
    return out.reshape(B, 1, 2 * M)
```

```python
import jax
import jax.numpy as jnp
from jax import lax
import jax.experimental.pallas as pl
import jax.experimental.pallas.tpu as pltpu

F32 = jnp.float32
BF16 = jnp.bfloat16
NT = (((1,), (1,)), ((), ()))
NN = (((1,), (0,)), ((), ()))

B = 4
H = 32
D = 128
M = 512
DC = 512
S = 4096
HKV = 8
NIT = 32
RING = 4
LAG = 2
OFF = 2
SH = 8
HI, LO = 0, 1
PRE = 4
SCALE = 0.08837890625

S_K, S_V, S_C, S_WQA, S_WUK, S_WQB, S_WUV, S_X, S_WOB, S_WOA, S_FIN, S_N = (
    0, 4, 8, 12, 13, 14, 15, 16, 18, 26, 34, 38)


def _dot(a, b, dims=NN):
    return lax.dot_general(a, b, dims, preferred_element_type=F32)


def _iota(shape, dim):
    return lax.broadcasted_iota(jnp.int32, shape, dim)


def _kernel(xa_hbm, ckv_hbm, wqa_hbm, wuk_hbm, wuv_hbm, woa_hbm,
            xb_hbm, k_hbm, v_hbm, wqb_hbm, wob_hbm,
            o_hbm,
            xa_v, xb_v, o_v, k_v, v_v, c_v, wqa_v, wuk_v, wuv_v, wqb_v, woa_v, wob_v,
            x2_s, r_s, qabs_s, qb_s, qg_s, og_s, ob_s,
            ma_s, la_s, acca_s, mb_s, lb_s, accb_s, lx_s, lo_s, w32_s, sem):

    def ds(start, n, align):
        if isinstance(start, int):
            return pl.ds(start, n)
        return pl.ds(pl.multiple_of(start, align), n)

    def rows(i, n):
        return ds(i * n, n, n)

    def go(src, dst, s, prio):
        pltpu.make_async_copy(src, dst, sem.at[s]).start(priority=prio)

    def wait_all(buf, s):
        pltpu.make_async_copy(buf, buf, sem.at[s]).wait()

    def loop(lo, hi, fn):
        def body(i, c):
            fn(i)
            return c
        lax.fori_loop(lo, hi, body, 0)

    def cp_n(src, dst, half, t, s, prio):
        g = pl.ds(half * 4, 4)
        go(src.at[g, rows(t, 16)], dst.at[g, rows(t, 16)], s, prio)

    def cp_q(half, t, prio):
        g, r, c = pl.ds(half * 4, 4), rows(t >> 4, 8), rows(t & 15, 256)
        go(wqb_hbm.at[g, r, c], wqb_v.at[g, r, c], S_WQB, prio)

    def tick_p1(t, hi=HI):
        for u in range(2):
            cp_n(wqa_hbm, wqa_v, 1, 2 * t + u, S_WQA, LO)
            cp_q(0, 2 * t + u, LO)
        cp_q(1, t, hi)

    def tick_p2(t):
        for u in range(2):
            cp_n(wqa_hbm, wqa_v, 0, 2 * t + u, S_WQA, LO)
            cp_n(wuk_hbm, wuk_v, 1, 2 * t + u, S_WUK, LO)
        cp_q(1, 64 + t, HI)

    def tick_p3(t):
        cp_n(wuk_hbm, wuk_v, 0, t, S_WUK, LO)
        cp_n(wuv_hbm, wuv_v, 1, t, S_WUV, LO)
        cp_n(wuv_hbm, wuv_v, 0, t, S_WUV, HI)

    def tick_main(i, j, wrap=False):
        s, w, p = i & (RING - 1), i >> 3, i & 7

        def cp(is_k, g0, n, d0, u, prio):
            src, dst, sm = (k_hbm, k_v, S_K) if is_k else (v_hbm, v_v, S_V)
            a = j * 64 + u * 16
            segs = [(p * 512 + a + SH, a, 16)]
            if isinstance(j, int) and a == 496:
                segs = [(p * 512 + a + SH, a, 16 - SH), ((p * 512 + 512) & (S - 1), 512 - SH, SH)]
            for rs, rd, nr in segs:
                go(src.at[pl.ds(g0, n), ds(rs, nr, 8)], dst.at[s, pl.ds(d0, n), ds(rd, nr, 8)],
                   sm + s, prio)

        for u in range(4):
            if not wrap:
                cp(False, w * 8 + OFF, 8, 0, u, LO)
                cp(True, w * 8 + OFF, 8, 0, u, HI)
            else:
                cp(False, 24 + OFF, 8 - OFF, 0, u, LO)
                cp(True, 0, OFF, 8 - OFF, u, LO)
                cp(True, 24 + OFF, 8 - OFF, 0, u, HI)
                cp(False, 0, OFF, 8 - OFF, u, HI)
        go(ckv_hbm.at[w, rows(64 + p * 8 + j, 32)], c_v.at[s, rows(8 + j, 32)], S_C + s, LO)
        go(ckv_hbm.at[w, rows(p * 8 + j, 32)], c_v.at[s, rows(j, 32)], S_C + s, HI)

    def issue_unit(i, wrap):
        loop(0, 7, lambda j: tick_main(i, j, wrap))
        tick_main(i, 7, wrap)

    def tick_e(t, late):
        if not late:
            r = rows(t >> 2, 32)
            go(wob_hbm.at[4 + (t & 3), r], wob_v.at[4 + (t & 3), r], S_WOB + 4 + (t >> 4), LO)
        else:
            fin = t >= 112
            q = jnp.where(fin, (t >> 2) & 3, t & 3)
            r = rows(jnp.where(fin, 12 + (t & 3), (t >> 2) & 15), 32)
            go(woa_hbm.at[q, r], woa_v.at[q, r], jnp.where(fin, S_FIN + q, S_WOA - 4 + (t >> 4)), LO)
        r, c = rows(t >> 1, 8), rows(t & 1, 256)
        go(woa_hbm.at[pl.ds(4, 4), r, c], woa_v.at[pl.ds(4, 4), r, c], S_WOA + 4 + (t >> 5), HI)
        go(wob_hbm.at[pl.ds(0, 4), r, c], wob_v.at[pl.ds(0, 4), r, c], S_WOB + (t >> 5), HI)

    tick_p1(0, LO)
    cxa = pltpu.make_async_copy(xa_hbm, xa_v, sem.at[S_X])
    cxb = pltpu.make_async_copy(xb_hbm, xb_v, sem.at[S_X + 1])
    cxa.start()
    cxb.start()
    loop(1, PRE, lambda t: tick_p1(t, LO))
    loop(PRE, 64, tick_p1)

    cxa.wait()
    cxb.wait()
    ex = (_iota((128, 256), 1) // 2 == _iota((128, 256), 0)).astype(BF16)
    par8 = (_iota((8, 256), 1) % 2) == (_iota((8, 256), 0) // 4)
    xa = xa_v[...].astype(F32)
    xa8 = jnp.concatenate([xa, xa], axis=0).astype(BF16)
    for n in range(4):
        t = jnp.where(par8, _dot(xa8[:, n * 128:(n + 1) * 128], ex), 0.0)
        x2_s[2 * n] = t[:, :128]
        x2_s[2 * n + 1] = t[:, 128:]

    def init(b):
        ma_s[b] = jnp.full(ma_s.shape[1:], -jnp.inf, F32)
        la_s[b] = jnp.zeros(la_s.shape[1:], F32)
        acca_s[b] = jnp.zeros(acca_s.shape[1:], F32)
        mb_s[b] = jnp.full(mb_s.shape[1:], -jnp.inf, F32)
        lb_s[b] = jnp.zeros(lb_s.shape[1:], F32)
        accb_s[b] = jnp.zeros(accb_s.shape[1:], F32)
        qb_s[rows(16 + b, 16), :] = jnp.zeros((16, 128), F32)
        og_s[ds(256 + 80 * b, 80, 8), :] = jnp.zeros((80, 128), F32)
    loop(0, B, init)
    w32_s[pl.ds(1024, 16), :] = jnp.zeros((16, 128), jnp.uint32)

    loop(0, 64, tick_p2)
    loop(0, 32, tick_p3)

    wait_all(wqb_v, S_WQB)
    xb = xb_v[...].astype(F32)
    xb8 = jnp.concatenate([xb, xb], axis=0).astype(BF16)

    def qb_job(j):
        loop(0, 4, lambda u: tick_p3(32 + 4 * j + u))
        q = _dot(xb8, wqb_v[:, :, rows(j, 512)].reshape(M, 512))
        for u in range(4):
            qb_s[rows(4 * j + u, 8), :] = q[:, u * 128:(u + 1) * 128]
    loop(0, 8, qb_job)
    for w in range(4):
        for r in range(8):
            g = (8 * w + OFF + r) % 32
            qg_s[w, pl.ds(r * 8, 8), :] = qb_s[pl.ds((g % 8) * 32 + g // 8, 8, stride=8), :]

    def stage(w_v, j):
        w32_s[pl.ds(0, 1024), :] = pltpu.bitcast(w_v[j], jnp.uint32)

    def tile(p):
        return pltpu.bitcast(w32_s[pl.ds(p, 64, stride=16), :], BF16)

    wait_all(wqa_v, S_WQA)

    def qa_job(j, acc):
        loop(0, 8, lambda u: tick_p3(64 + 8 * j + u))
        stage(wqa_v, j)
        w = jnp.concatenate([tile(p) for p in range(16)], axis=1)
        return acc + _dot(x2_s[j].astype(BF16), w)
    qa = lax.fori_loop(0, 8, qa_job, jnp.zeros((8, 2048), F32)).astype(BF16)

    loop(0, 8, lambda j: tick_main(0, j))

    wait_all(wuk_v, S_WUK)
    parw = (_iota((128, 128), 1) % 2) == ((_iota((128, 128), 0) // 4) % 2)

    def qabs_job(j):
        tick_main(1, j)
        stage(wuk_v, j)
        r = [_dot(qa[:, p * 128:(p + 1) * 128], tile(p), NT) for p in range(16)]
        r_s[j] = jnp.where(parw, jnp.concatenate(r, axis=0), 0.0).astype(BF16)
    loop(0, 8, qabs_job)

    cmp = (_iota((256, 128), 0) // 2 == _iota((256, 128), 1)).astype(BF16)
    perm = ((_iota((128, 128), 0) % 32) * 4 + _iota((128, 128), 0) // 32
            == _iota((128, 128), 1)).astype(BF16)

    def pack_job(n):
        t = _dot(jnp.concatenate([r_s[2 * n], r_s[2 * n + 1]], axis=1), cmp).astype(BF16)
        qabs_s[n] = _dot(perm, t).astype(BF16)
    loop(0, 4, pack_job)

    def online(sc, m_s, l_s, b):
        sc = (sc.astype(BF16).astype(F32) * SCALE).astype(BF16).astype(F32)
        m_old = m_s[b]
        m_new = jnp.maximum(m_old, jnp.max(sc, axis=-1, keepdims=True))
        alpha = jnp.exp(m_old - m_new)
        p = jnp.exp(sc - jnp.tile(m_new, (1, 4)))
        l_s[b] = alpha * l_s[b] + ((p[:, 0:128] + p[:, 128:256]) + (p[:, 256:384] + p[:, 384:512]))
        m_s[b] = m_new
        return p, alpha

    def main(i):
        @pl.when(i < 24 - LAG)
        def _():
            issue_unit(i + LAG, False)

        @pl.when(jnp.logical_and(i >= 24 - LAG, i < NIT - LAG))
        def _():
            issue_unit(i + LAG, True)

        @pl.when(i >= NIT - LAG)
        def _():
            loop(0, 27, lambda u: tick_e((i - (NIT - LAG)) * 27 + u, False))

        @pl.when(i < 8)
        def _():
            stage(wuv_v, i)
            for p in range(16):
                wuv_v[i, pl.ds(p * 128, 128), :] = tile(p)

        s, b = i & (RING - 1), i >> 3
        wait_all(k_v.at[s], S_K + s)
        wait_all(v_v.at[s], S_V + s)
        wait_all(c_v.at[s], S_C + s)
        sc = [_dot(qg_s[b, pl.ds(g * 8, 8), :].astype(BF16), k_v[s, g], NT) for g in range(HKV)]
        p, alpha = online(jnp.concatenate(sc, axis=0), mb_s, lb_s, b)

        q = jnp.concatenate([qabs_s[n, rows(b, 32), :] for n in range(4)], axis=1)
        pa, alpha_a = online(_dot(q, c_v[s], NT), ma_s, la_s, b)

        o = [_dot(p[g * 8:(g + 1) * 8].astype(BF16), v_v[s, g]) for g in range(HKV)]
        accb_s[b] = accb_s[b] * alpha + jnp.concatenate(o, axis=0)
        acca_s[b] = acca_s[b] * jnp.tile(alpha_a, (1, 4)) + _dot(pa.astype(BF16), c_v[s])

    wait_all(wuv_v, S_WUV)
    loop(0, NIT, main)

    loop(54, 64, lambda t: tick_e(t, False))
    for b in range(B):
        o = accb_s[b] / jnp.sum(lb_s[b], axis=-1, keepdims=True)
        if b < 3:
            og_s[pl.ds(b * 64 + OFF * 8, 64), :] = o
        else:
            og_s[pl.ds(192 + OFF * 8, 64 - OFF * 8), :] = o[:64 - OFF * 8]
            og_s[pl.ds(0, OFF * 8), :] = o[64 - OFF * 8:]
        acca_s[b] = acca_s[b] / jnp.sum(la_s[b], axis=-1, keepdims=True)
    for h in range(H):
        ob_s[(h // 16) * 4 + h % 4, :, pl.ds((h // 4) % 4 * 128, 128)] = (
            og_s[pl.ds((h // 4) * 8 + h % 4, 8, stride=64), :])

    permt = ((_iota((128, 128), 1) % 32) * 4 + _iota((128, 128), 1) // 32
             == _iota((128, 128), 0)).astype(BF16)
    par128 = (_iota((128, 256), 1) % 2) == ((_iota((128, 256), 0) // 4) % 2)

    def expand_job(n):
        loop(0, 4, lambda u: tick_e(64 + 4 * n + u, True))
        cc = acca_s[:, :, rows(n, 128)].reshape(128, 128).astype(BF16)
        t = jnp.where(par128, _dot(_dot(permt, cc).astype(BF16), ex), 0.0)
        lx_s[2 * n] = t[:, :128]
        lx_s[2 * n + 1] = t[:, 128:]
    loop(0, 4, expand_job)

    def ctx_job(j, acc):
        loop(0, 3, lambda u: tick_e(80 + 3 * j + u, True))
        return acc + jnp.concatenate(
            [_dot(lx_s[j, pl.ds(p * 8, 8), :].astype(BF16), wuv_v[j, pl.ds(p * 128, 128), :])
             for p in range(16)], axis=0)
    ctx = lax.fori_loop(0, 8, ctx_job, jnp.zeros((128, 128), F32))
    top = _iota((8, 128), 0) < 4
    for h in range(H):
        c = ctx[(h // 2) * 8:(h // 2) * 8 + 8]
        if h < 16 and h % 4 == 3:
            c = jnp.concatenate([c[4:], c[:4]], axis=0)
        else:
            c = jnp.where(top, c, 0.0) if h % 2 == 0 else jnp.where(top, 0.0, c)
        lo_s[(h // 16) * 4 + h % 4, :, pl.ds((h // 4) % 4 * 128, 128)] = c

    def arrive(w_v, k, s):
        wait_all(w_v.at[pl.ds(k & 4, 4), rows(k & 3, 128)], s + k)

    def proj(lhs_s, w_v, k):
        w = w_v[pl.ds(k & 4, 4), rows(k & 3, 128), :]
        return _dot(lhs_s[k].astype(BF16), w.reshape(512, M))

    def wo_job(n, carry):
        @pl.when(n < 3)
        def _():
            loop(0, 8, lambda u: tick_e(104 + 8 * n + u, True))

        ka = (0x710654 >> (4 * n)) & 7
        kb = (0x327615 >> (4 * n)) & 7
        arrive(wob_v, kb, S_WOB)
        arrive(woa_v, ka, S_WOA)
        return carry[0] + proj(lo_s, woa_v, ka), carry[1] + proj(ob_s, wob_v, kb)
    arrive(wob_v, 0, S_WOB)
    arrive(wob_v, 4, S_WOB)
    outa, outb = lax.fori_loop(
        0, 6, wo_job, (jnp.zeros((8, M), F32), proj(ob_s, wob_v, 0) + proj(ob_s, wob_v, 4)))
    arrive(woa_v, 2, S_WOA)
    outa = outa + proj(lo_s, woa_v, 2)
    o_v[:, M:] = outb[0:4].astype(BF16)
    outa = outa + jnp.concatenate([outa[4:], outa[:4]], axis=0)

    def fin_job(q, acc):
        blk = woa_v.at[q, pl.ds(384, 128)]
        lhs = lo_s[3, :, rows(q, 128)].astype(BF16)
        wait_all(blk, S_FIN + q)
        return acc + _dot(lhs, blk[...])
    outa = lax.fori_loop(0, 4, fin_job, outa)
    o_v[:, :M] = outa[0:4].astype(BF16)
    co = pltpu.make_async_copy(o_v, o_hbm, sem.at[S_X])
    co.start()
    co.wait()


@jax.jit
def pallas_concat_heads__compressed_kv_cla__gqa_block_cached__decode_kernel(
    A_x: jax.Array,
    A_c_kv: jax.Array,
    A_w_q: jax.Array,
    A_w_uk: jax.Array,
    A_w_uv: jax.Array,
    A_w_o: jax.Array,
    B_x: jax.Array,
    B_k_cache: jax.Array,
    B_v_cache: jax.Array,
    B_wq: jax.Array,
    B_wo: jax.Array,
):
    args = (
        A_x.reshape(B, M),
        A_c_kv,
        A_w_q.reshape(8, 2048, D),
        A_w_uk.reshape(8, 2048, D),
        A_w_uv.reshape(8, 2048, D),
        A_w_o.reshape(8, 512, M),
        B_x.reshape(B, M),
        B_k_cache.reshape(B * HKV, S, D),
        B_v_cache.reshape(B * HKV, S, D),
        B_wq.reshape(8, 64, H * D),
        B_wo.reshape(8, 512, M),
    )
    V = pltpu.VMEM
    scratch = [
        V((B, M), BF16), V((B, M), BF16), V((B, 2 * M), BF16),
        V((RING, HKV, 512, D), BF16), V((RING, HKV, 512, D), BF16), V((RING, 512, DC), BF16),
        V((8, 2048, D), BF16), V((8, 2048, D), BF16), V((8, 2048, D), BF16),
        V((8, 64, H * D), BF16), V((8, 512, M), BF16), V((8, 512, M), BF16),
        V((8, 8, 128), F32),
        V((8, 128, 128), BF16),
        V((4, 128, 128), BF16),
        V((256 + 64, D), F32),
        V((B, 64, D), F32),
        V((256 + 320, D), F32),
        V((8, 8, 512), F32),
        V((B, H, 128), F32), V((B, H, 128), F32), V((B, H, DC), F32),
        V((B, 64, 128), F32), V((B, 64, 128), F32), V((B, 64, D), F32),
        V((8, 128, 128), F32),
        V((8, 8, 512), F32),
        V((1040, 128), jnp.uint32),
        pltpu.SemaphoreType.DMA((S_N,)),
    ]
    out = pl.pallas_call(
        _kernel,
        in_specs=[pl.BlockSpec(memory_space=pl.ANY)] * 11,
        out_specs=pl.BlockSpec(memory_space=pl.ANY),
        out_shape=jax.ShapeDtypeStruct((B, 2 * M), BF16),
        scratch_shapes=scratch,
        compiler_params=pltpu.CompilerParams(
            vmem_limit_bytes=64 * 1024 * 1024,
            disable_bounds_checks=True,
            disable_semaphore_checks=True,
        ),
    )(*args)
    return out.reshape(B, 1, 2 * M)
```
